```python
import jax
import jax.numpy as jnp

def _softmax(x, axis=-1):
    return jax.nn.softmax(x, axis=axis)

def _gelu(x):
    return jax.nn.gelu(x, approximate=True)

def _silu(x):
    return jax.nn.silu(x)

def _sigmoid(x):
    return jax.nn.sigmoid(x)

def _layernorm(x, axis=-1, eps=1e-05):
    m = jnp.mean(x, axis=axis, keepdims=True)
    v = jnp.var(x, axis=axis, keepdims=True)
    return (x - m) / jnp.sqrt(v + eps)

def _scatter_add(tgt, idx, src, axis=0):
    return tgt.at[idx].add(src)

def _segment_sum(src, seg, n):
    return jax.ops.segment_sum(src, seg, n)

class _Rng:

    def __init__(self, key):
        self._k = key

    def _next(self):
        self._k, sub = jax.random.split(self._k)
        return sub

    def normal(self, shape):
        return jax.random.normal(self._next(), shape, dtype=jnp.bfloat16)

    def randint(self, lo, hi, shape):
        return jax.random.randint(self._next(), shape, lo, hi, dtype=jnp.int32)

    def uniform(self, shape, lo=0.0, hi=1.0):
        return jax.random.uniform(self._next(), shape, jnp.bfloat16, lo, hi)

    def permutation(self, n):
        return jax.random.permutation(self._next(), n)
kernel_name = 'standalone__window_attn_davit__vision'

def setup_inputs():
    _rng = _Rng(jax.random.key(int.from_bytes(__import__("os").urandom(4), "little")))
    _w = lambda a: (lambda t: t.astype(jnp.bfloat16) if jnp.issubdtype(t.dtype, jnp.floating) else t)(jnp.asarray(a))
    HW = 512
    C0 = 192
    ws = 7
    nh = 4
    H = W = max(HW // ws * ws, ws)
    C = max(C0 // nh * nh, nh)
    k = 3
    return {'x': _w((lambda *s: _rng.normal(s) * 0.05)(1, H, W, C)), 'dw_pe': _w((lambda *s: _rng.normal(s) * 0.05)(k, k, C) * 0.1), 'w_qkv': _w((lambda *s: _rng.normal(s) * 0.05)(C, 3 * C) * C ** (-0.5)), 'w_o': _w((lambda *s: _rng.normal(s) * 0.05)(C, C) * C ** (-0.5))}

def reference(x, dw_pe, w_qkv, w_o):
    B, H, W, C = x.shape
    ws = 7
    nh = 4
    dh = C // nh
    kk = dw_pe.shape[0]
    pad = kk // 2
    xp = jnp.pad(x, ((0, 0), (pad, pad), (pad, pad), (0, 0)))
    pe = jnp.zeros_like(x)
    for i in range(kk):
        for j in range(kk):
            pe = pe + xp[:, i:i + H, j:j + W, :] * dw_pe[i, j][None, None, None, :]
    x0 = x + pe
    h = _layernorm(x0, axis=-1)
    hw = h.reshape(B, H // ws, ws, W // ws, ws, C)
    hw = (lambda x, *d: x.transpose(*d))(hw, 0, 1, 3, 2, 4, 5)
    hw = hw.reshape(-1, ws * ws, C)
    qkv = (hw @ w_qkv).reshape(-1, ws * ws, 3, nh, dh)
    q = qkv[:, :, 0].copy()
    k = qkv[:, :, 1].copy()
    v = qkv[:, :, 2].copy()
    scale = dh ** (-0.5)
    attn = jnp.einsum('wnhd,wmhd->whnm', q, k) * scale
    attn = _softmax(attn, axis=-1)
    out = jnp.einsum('whnm,wmhd->wnhd', attn, v)
    out = out.reshape(-1, ws * ws, C) @ w_o
    out = out.reshape(B, H // ws, W // ws, ws, ws, C)
    out = (lambda x, *d: x.transpose(*d))(out, 0, 1, 3, 2, 4, 5)
    out = out.reshape(B, H, W, C)
    return x0 + out
```

```python
import functools

import jax
import jax.numpy as jnp
import jax.experimental.pallas as pl
import jax.experimental.pallas.tpu as pltpu
import numpy as np

_WS = 7
_NH = 4
_NN = (((1,), (0,)), ((), ()))
_NT = (((1,), (1,)), ((), ()))
_F32 = jnp.float32
_BF16 = jnp.bfloat16
_NEG = -1e30
_UNROLL = 2


def _dot(a, b, dims):
    return jax.lax.dot_general(a, b, dims, preferred_element_type=_F32)


def _xpose(a):
    r, c = a.shape
    rp, cp = -(-r // 128) * 128, -(-c // 128) * 128
    if rp != r:
        a = jnp.concatenate([a, jnp.zeros((rp - r, c), a.dtype)], axis=0)
    if cp != c:
        a = jnp.concatenate([a, jnp.zeros((rp, cp - c), a.dtype)], axis=1)
    return a.T[:c, :r]


def _pk(a):
    return pltpu.bitcast(a.astype(_BF16), jnp.uint32)


def _upk(a):
    return pltpu.bitcast(a, _BF16)


def _kernel(x_ref, xu_ref, xd_ref, dw_ref, wqkv_ref, wo_ref, o_ref,
            wconv_s, lab_s, lba_s, rk_s, loe_s, loo_s,
            xs_s, x0_s, h_s, k_s, oe_s, oo_s, q_s, v_s, p_s, r_s, *, H, W, C, nstrips):
    t = pl.program_id(0)
    dh = C // _NH
    WP = 512
    nwin = W // _WS
    npair = (nwin + 1) // 2
    CH = 48
    nunit = _WS * (C // CH)
    bufB = jax.lax.rem(t, 2)
    bufA = 1 - bufB

    @pl.when(t == 0)
    def _prep():
        def padk(a):
            return jnp.concatenate([a, jnp.zeros((a.shape[0], 256 - C), _F32)], axis=1)
        wT = _xpose(wqkv_ref[...].astype(_F32))
        lab_s[...] = _pk(padk(jnp.concatenate(
            [wT[0:dh], wT[2 * dh:3 * dh], wT[2 * C:2 * C + 2 * dh]], axis=0)))
        lba_s[...] = _pk(padk(jnp.concatenate(
            [wT[dh:2 * dh], wT[3 * dh:4 * dh], wT[2 * C + 2 * dh:3 * C]], axis=0)))
        z = jnp.zeros((128 - 2 * dh, C), _F32)
        kscale = float(dh) ** -0.5 * float(np.log2(np.e))
        k01 = jnp.concatenate([wT[C:C + 2 * dh] * kscale, z], axis=0)
        k23 = jnp.concatenate([wT[C + 2 * dh:2 * C] * kscale, z], axis=0)
        rk_s[...] = _pk(jnp.concatenate([padk(k01).T, padk(k23).T], axis=1))
        wo = wo_ref[...].astype(_F32)
        woe = jnp.concatenate([wo[0:dh], wo[2 * dh:3 * dh], z], axis=0)
        woo = jnp.concatenate([wo[dh:2 * dh], wo[3 * dh:4 * dh], z], axis=0)
        loe_s[...] = _pk(_xpose(woe))
        loo_s[...] = _pk(_xpose(woo))
        dwT = _xpose(dw_ref[...].astype(_F32))
        for k in range(9):
            wk = jnp.broadcast_to(dwT[0:C, k:k + 1], (C, 128))
            wconv_s[k] = wk + 1.0 if k == 4 else wk
        h_s[:, :, :, pl.ds(WP, 8), :] = jnp.zeros((2, 2, _WS, 8, 128), _F32)
        k_s[:, :, :, pl.ds(WP, 8), :] = jnp.zeros((2, 2, _WS, 8, 128), _F32)
        x0_s[...] = jnp.zeros(x0_s.shape, _F32)
        oe_s[...] = jnp.zeros(oe_s.shape, _F32)
        oo_s[...] = jnp.zeros(oo_s.shape, _F32)

    lane = jax.lax.broadcasted_iota(jnp.int32, (1, 128), 1)
    last_ok = lane < (W - (WP - 128))

    def stage_row(dst, v, ok):
        v = v.astype(_F32)
        okl = last_ok if ok is None else jnp.logical_and(last_ok, ok)
        lo = v[:, :WP - 128] if ok is None else jnp.where(ok, v[:, :WP - 128], 0.0)
        xs_s[dst, :, :WP - 128] = lo
        xs_s[dst, :, WP - 128:] = jnp.where(okl, v[:, WP - 128:], 0.0)

    def conv_unit(u):
        r = u // (C // CH)
        c0 = pl.multiple_of((u - r * (C // CH)) * CH, CH)
        y = [None, None, None]
        for a in range(3):
            xv = xs_s[r + a, pl.ds(c0, CH), :]
            for b in range(3):
                w = wconv_s[3 * a + b, pl.ds(c0, CH), :]
                term = xv * jnp.concatenate([w] * (WP // 128), axis=1)
                y[b] = term if y[b] is None else y[b] + term
        x0 = y[1] + (pltpu.roll(y[0], 1, 1) + pltpu.roll(y[2], WP - 1, 1))
        for j in range(WP // 128):
            x0_s[bufA, r, j, pl.ds(c0, CH), :] = x0[:, 128 * j:128 * (j + 1)]

    def norm_unit(r, j):
        x0 = x0_s[bufA, r, j]
        mean = jnp.sum(x0, axis=0, keepdims=True) * (1.0 / C)
        ex2 = jnp.sum(x0 * x0, axis=0, keepdims=True) * (1.0 / C)
        rstd = jax.lax.rsqrt(jnp.maximum(ex2 - mean * mean, 0.0) + 1e-5)
        hn = (x0 - mean) * rstd
        hb = jnp.concatenate([hn, jnp.zeros((256 - C, 128), _F32)], axis=0).astype(_BF16).T
        hf = hb.astype(_F32)
        h_s[bufA, 0, r, 128 * j:128 * (j + 1), :] = hf[:, 0:128]
        h_s[bufA, 1, r, 128 * j:128 * (j + 1), :] = hf[:, 128:256]
        kk = _dot(hb, _upk(rk_s[...]), _NN)
        k_s[bufA, 0, r, 128 * j:128 * (j + 1), :] = kk[:, 0:128]
        k_s[bufA, 1, r, 128 * j:128 * (j + 1), :] = kk[:, 128:256]

    def out_unit(r, j):
        sl = slice(128 * j, 128 * (j + 1))
        y = (_dot(_upk(loe_s[...]), oe_s[r, sl, :].astype(_BF16), _NT)
             + _dot(_upk(loo_s[...]), oo_s[r, sl, :].astype(_BF16), _NT))
        o_ref[r, :, sl] = (x0_s[bufB, r, j] + y).astype(o_ref.dtype)

    left = lane < 64
    mL = jnp.where(left, jnp.uint32(0xFFFFFFFF), jnp.uint32(0))
    mR = jnp.where(left, jnp.uint32(0), jnp.uint32(0xFFFFFFFF))
    key_ok = (jax.lax.broadcasted_iota(jnp.int32, (56, 128), 0) % 8) < _WS
    z8 = jnp.zeros((8, 256), _F32)
    z32 = jnp.zeros((32, 128), _F32)
    z8l = jnp.zeros((8, 128), _F32)

    def softmax_t(s):
        s = jnp.where(key_ok, s, _NEG)
        m = jnp.max(s, axis=0, keepdims=True)
        p = jnp.exp2(s - m)
        l = jnp.sum(p, axis=0, keepdims=True)
        return p, pl.reciprocal(l, approx=False)

    def gather(ref, t0):
        return [jnp.concatenate([ref[bufB, k, r, pl.ds(t0, 8), :] for r in range(_WS)], axis=0)
                for k in range(2)]

    def proj(p, slot):
        ta_ = p * (2 * _WS)
        hA = jnp.concatenate(gather(h_s, ta_), axis=1)
        hB = jnp.concatenate(gather(h_s, ta_ + _WS), axis=1)
        hAB = jnp.concatenate([hA, z8, hB, z8], axis=0).astype(_BF16)
        hBA = jnp.concatenate([hB, z8, hA, z8], axis=0).astype(_BF16)
        r1 = _pk(_dot(_upk(lab_s[...]), hAB, _NT))
        r2 = _pk(_dot(_upk(lba_s[...]), hBA, _NT))
        qe, qo = r1[0:dh], r2[0:dh]
        for t2 in range(2):
            e = qe[(dh // 2) * t2:(dh // 2) * (t2 + 1)]
            o = qo[(dh // 2) * t2:(dh // 2) * (t2 + 1)]
            q_s[slot, 2 * t2] = jnp.concatenate([e & mL, o & mR], axis=0)
            q_s[slot, 2 * t2 + 1] = jnp.concatenate([e & mR, o & mL], axis=0)
        v_s[slot, 0:dh, :] = r1[dh:2 * dh]
        v_s[slot, dh:2 * dh, :] = r2[dh:2 * dh]

    def scores(p, slot):
        ta_ = p * (2 * _WS)
        kA = gather(k_s, ta_)
        kB = gather(k_s, ta_ + _WS)
        out = []
        for t2 in range(2):
            sA = _dot(kA[t2][:, 0:96], _upk(q_s[slot, 2 * t2]), _NN)
            sB = _dot(kB[t2][:, 0:96], _upk(q_s[slot, 2 * t2 + 1]), _NN)
            out.append((sA, sB))
        return out

    def probs(ss, slot):
        for t2 in range(2):
            pA, rA = softmax_t(ss[t2][0])
            pB, rB = softmax_t(ss[t2][1])
            uA = _pk(jnp.concatenate([pA, z8l], axis=0))
            uB = _pk(jnp.concatenate([pB, z8l], axis=0))
            pe, po = [uA & mL, uB & mR], [uA & mR, uB & mL]
            if t2 == 1:
                pe, po = pe[::-1], po[::-1]
            p_s[slot, 2 * t2] = jnp.concatenate(pe, axis=0)
            p_s[slot, 2 * t2 + 1] = jnp.concatenate(po, axis=0)
            r_s[slot, 2 * t2] = jnp.broadcast_to(jnp.where(left, rA, rB), (8, 128))
            r_s[slot, 2 * t2 + 1] = jnp.broadcast_to(jnp.where(left, rB, rA), (8, 128))

    def pv(p, slot):
        ta_ = p * (2 * _WS)
        tb_ = ta_ + _WS
        oe, oo = [], []
        for t2 in range(2):
            v2 = _upk(v_s[slot, dh * t2:dh * (t2 + 1), :])
            oe.append(_dot(v2[0:dh], _upk(p_s[slot, 2 * t2]), _NN) * r_s[slot, 2 * t2, 0:1, :])
            oo.append(_dot(v2[dh:2 * dh], _upk(p_s[slot, 2 * t2 + 1]), _NN)
                      * r_s[slot, 2 * t2 + 1, 0:1, :])
        oeT = jnp.concatenate(oe + [z32], axis=0).astype(_BF16).T.astype(_F32)
        ooT = jnp.concatenate(oo + [z32], axis=0).astype(_BF16).T.astype(_F32)
        for r in range(_WS):
            oe_s[r, pl.ds(ta_, 8), :] = oeT[8 * r:8 * r + 8]
            oo_s[r, pl.ds(ta_, 8), :] = ooT[64 + 8 * r:64 + 8 * r + 8]
        for r in range(_WS):
            oe_s[r, pl.ds(tb_, 8), :] = oeT[64 + 8 * r:64 + 8 * r + 8]
            oo_s[r, pl.ds(tb_, 8), :] = ooT[8 * r:8 * r + 8]

    def iteration(p, conv=True):
        s0 = jax.lax.rem(p, 3)
        s1 = jax.lax.rem(p + 1, 3)
        s2 = jax.lax.rem(p + 2, 3)
        ss = scores(p + 1, s1)
        pv(p, s0)
        proj(jnp.minimum(p + 2, npair - 1), s2)
        probs(ss, s1)
        if conv:
            conv_unit(p)

    @pl.when(t > 0)
    def _attend():
        proj(0, 0)
        proj(1, 1)
        probs(scores(0, 0), 0)

        def body_x(i, carry):
            for k in range(_UNROLL):
                iteration(i * _UNROLL + k)
            return carry

        def body_x2(i, carry):
            for k in range(_UNROLL):
                iteration(i * _UNROLL + k, conv=False)
            return carry

        jax.lax.fori_loop(0, nunit // _UNROLL, body_x, 0)
        jax.lax.fori_loop(nunit // _UNROLL, (npair - 1) // _UNROLL, body_x2, 0)
        pv(npair - 1, (npair - 1) % 3)

    stage_row(0, xu_ref[0], t > 0)
    stage_row(_WS + 1, xd_ref[0], t < nstrips - 1)

    def body_y(r, carry):
        stage_row(r + 1, x_ref[r], None)
        for j in range(WP // 128):
            norm_unit(r, j)
            out_unit(r, j)
        return carry

    jax.lax.fori_loop(0, _WS, body_y, 0)


@jax.jit
def pallas_standalone__window_attn_davit__vision_kernel(x, dw_pe, w_qkv, w_o):
    B, H, W, C = x.shape
    assert B == 1 and H % _WS == 0 and W % _WS == 0 and W + _WS + 1 <= 520 and C == 192
    nstrips = H // _WS
    WP = 512
    u32 = jnp.uint32
    xt = jnp.transpose(x, (0, 1, 3, 2)).reshape(H, C, W)
    dw = jnp.pad(dw_pe.reshape(9, C), ((0, 7), (0, 256 - C)))
    kern = functools.partial(_kernel, H=H, W=W, C=C, nstrips=nstrips)

    def strip(t):
        return jnp.minimum(t, nstrips - 1)

    out = pl.pallas_call(
        kern,
        grid=(nstrips + 2,),
        in_specs=[
            pl.BlockSpec((_WS, C, WP), lambda t: (strip(t), 0, 0)),
            pl.BlockSpec((1, C, WP), lambda t: (jnp.maximum(strip(t) * _WS - 1, 0), 0, 0)),
            pl.BlockSpec((1, C, WP), lambda t: (jnp.minimum(strip(t) * _WS + _WS, H - 1), 0, 0)),
            pl.BlockSpec((16, 256), lambda t: (0, 0)),
            pl.BlockSpec((C, 3 * C), lambda t: (0, 0)),
            pl.BlockSpec((C, C), lambda t: (0, 0)),
        ],
        out_specs=pl.BlockSpec((_WS, C, WP), lambda t: (jnp.maximum(t - 2, 0), 0, 0)),
        out_shape=jax.ShapeDtypeStruct((H, C, W), x.dtype),
        scratch_shapes=[
            pltpu.VMEM((9, C, 128), _F32),
            pltpu.VMEM((96, 256), u32),
            pltpu.VMEM((96, 256), u32),
            pltpu.VMEM((128, 256), u32),
            pltpu.VMEM((C // 2, 128), u32),
            pltpu.VMEM((C // 2, 128), u32),
            pltpu.VMEM((_WS + 2, C, WP), _F32),
            pltpu.VMEM((2, _WS, WP // 128, C, 128), _F32),
            pltpu.VMEM((2, 2, _WS, WP + 8, 128), _F32),
            pltpu.VMEM((2, 2, _WS, WP + 8, 128), _F32),
            pltpu.VMEM((_WS, WP + 8, 128), _F32),
            pltpu.VMEM((_WS, WP + 8, 128), _F32),
            pltpu.VMEM((3, 4, 48, 128), u32),
            pltpu.VMEM((3, 96, 128), u32),
            pltpu.VMEM((3, 4, 64, 128), u32),
            pltpu.VMEM((3, 4, 8, 128), _F32),
        ],
        compiler_params=pltpu.CompilerParams(
            dimension_semantics=("arbitrary",),
            vmem_limit_bytes=64 * 1024 * 1024,
        ),
    )(xt, xt, xt, dw, w_qkv, w_o)
    return jnp.transpose(out.reshape(1, H, C, W), (0, 1, 3, 2))
```

```python
import functools

import jax
import jax.numpy as jnp
import jax.experimental.pallas as pl
import jax.experimental.pallas.tpu as pltpu
import numpy as np

_WS = 7
_NH = 4
_NN = (((1,), (0,)), ((), ()))
_NT = (((1,), (1,)), ((), ()))
_F32 = jnp.float32
_BF16 = jnp.bfloat16
_NEG = -1e30
_GROUP = 2
_CUNITS = 2
_NORM0 = 1


def _dot(a, b, dims):
    return jax.lax.dot_general(a, b, dims, preferred_element_type=_F32)


def _xpose(a):
    r, c = a.shape
    rp, cp = -(-r // 128) * 128, -(-c // 128) * 128
    if rp != r:
        a = jnp.concatenate([a, jnp.zeros((rp - r, c), a.dtype)], axis=0)
    if cp != c:
        a = jnp.concatenate([a, jnp.zeros((rp, cp - c), a.dtype)], axis=1)
    return a.T[:c, :r]


def _pk(a):
    return pltpu.bitcast(a.astype(_BF16), jnp.uint32)


def _upk(a):
    return pltpu.bitcast(a, _BF16)


def _kernel(x_ref, xu_ref, xd_ref, dw_ref, wqkv_ref, wo_ref, o_ref,
            wconv_s, lab_s, lba_s, rk_s, loe_s, loo_s,
            xs_s, x0_s, h_s, k_s, oe_s, oo_s, q_s, v_s, p_s, r_s, *, H, W, C, nstrips):
    t = pl.program_id(0)
    dh = C // _NH
    WP = 512
    nwin = W // _WS
    npair = (nwin + 1) // 2
    CH = 48
    nunit = _WS * (C // CH)
    bufB = jax.lax.rem(t, 2)
    bufA = 1 - bufB

    @pl.when(t == 0)
    def _prep():
        def padk(a):
            return jnp.concatenate([a, jnp.zeros((a.shape[0], 256 - C), _F32)], axis=1)
        wT = _xpose(wqkv_ref[...].astype(_F32))
        lab_s[...] = _pk(padk(jnp.concatenate(
            [wT[0:dh], wT[2 * dh:3 * dh], wT[2 * C:2 * C + 2 * dh]], axis=0)))
        lba_s[...] = _pk(padk(jnp.concatenate(
            [wT[dh:2 * dh], wT[3 * dh:4 * dh], wT[2 * C + 2 * dh:3 * C]], axis=0)))
        z = jnp.zeros((128 - 2 * dh, C), _F32)
        kscale = float(dh) ** -0.5 * float(np.log2(np.e))
        k01 = jnp.concatenate([wT[C:C + 2 * dh] * kscale, z], axis=0)
        k23 = jnp.concatenate([wT[C + 2 * dh:2 * C] * kscale, z], axis=0)
        rk_s[...] = _pk(jnp.concatenate([padk(k01).T, padk(k23).T], axis=1))
        wo = wo_ref[...].astype(_F32)
        woe = jnp.concatenate([wo[0:dh], wo[2 * dh:3 * dh], z], axis=0)
        woo = jnp.concatenate([wo[dh:2 * dh], wo[3 * dh:4 * dh], z], axis=0)
        loe_s[...] = _pk(_xpose(woe))
        loo_s[...] = _pk(_xpose(woo))
        dwT = _xpose(dw_ref[...].astype(_F32))
        for k in range(9):
            wk = jnp.broadcast_to(dwT[0:C, k:k + 1], (C, 128))
            wconv_s[k] = wk + 1.0 if k == 4 else wk
        h_s[1, :, :, pl.ds(WP, 8), :] = jnp.zeros((2, _WS, 8, 128), _F32)
        k_s[1, :, :, pl.ds(WP, 8), :] = jnp.zeros((2, _WS, 8, 128), _F32)
        h_s[0] = jnp.zeros(h_s.shape[1:], _F32)
        k_s[0] = jnp.zeros(k_s.shape[1:], _F32)
        xs_s[...] = jnp.zeros(xs_s.shape, _F32)
        x0_s[...] = jnp.zeros(x0_s.shape, _F32)
        oe_s[...] = jnp.zeros(oe_s.shape, _F32)
        oo_s[...] = jnp.zeros(oo_s.shape, _F32)

    lane = jax.lax.broadcasted_iota(jnp.int32, (1, 128), 1)
    last_ok = lane < (W - (WP - 128))

    def stage_row(dst, ref, ok, src=0):
        v = ref[src].astype(_F32)
        okl = last_ok if ok is None else jnp.logical_and(last_ok, ok)
        lo = v[:, :WP - 128] if ok is None else jnp.where(ok, v[:, :WP - 128], 0.0)
        xs_s[dst, :, :WP - 128] = lo
        xs_s[dst, :, WP - 128:] = jnp.where(okl, v[:, WP - 128:], 0.0)

    def conv_unit(u):
        r = u // (C // CH)
        c0 = (u - r * (C // CH)) * CH
        y = [None, None, None]
        for a in range(3):
            xv = xs_s[r + a, c0:c0 + CH, :]
            for b in range(3):
                w = wconv_s[3 * a + b, c0:c0 + CH, :]
                term = xv * jnp.concatenate([w] * (WP // 128), axis=1)
                y[b] = term if y[b] is None else y[b] + term
        x0 = y[1] + (pltpu.roll(y[0], 1, 1) + pltpu.roll(y[2], WP - 1, 1))
        for j in range(WP // 128):
            x0_s[bufA, r, j, c0:c0 + CH, :] = x0[:, 128 * j:128 * (j + 1)]

    def norm_unit(r, j):
        x0 = x0_s[bufA, r, j]
        mean = jnp.sum(x0, axis=0, keepdims=True) * (1.0 / C)
        ex2 = jnp.sum(x0 * x0, axis=0, keepdims=True) * (1.0 / C)
        rstd = jax.lax.rsqrt(jnp.maximum(ex2 - mean * mean, 0.0) + 1e-5)
        hn = (x0 - mean) * rstd
        hb = jnp.concatenate([hn, jnp.zeros((256 - C, 128), _F32)], axis=0).astype(_BF16).T
        hf = hb.astype(_F32)
        h_s[bufA, 0, r, 128 * j:128 * (j + 1), :] = hf[:, 0:128]
        h_s[bufA, 1, r, 128 * j:128 * (j + 1), :] = hf[:, 128:256]
        kk = _dot(hb, _upk(rk_s[...]), _NN)
        k_s[bufA, 0, r, 128 * j:128 * (j + 1), :] = kk[:, 0:128]
        k_s[bufA, 1, r, 128 * j:128 * (j + 1), :] = kk[:, 128:256]

    def out_unit(r, j):
        sl = slice(128 * j, 128 * (j + 1))
        oe = oe_s[r, sl, :].astype(_BF16)
        oo = oo_s[r, sl, :].astype(_BF16)
        for m in range(2):
            a0, b0 = 48 * m, 96 * m
            y = (_dot(_upk(loe_s[a0:a0 + 48, :]), oe, _NT) + _dot(_upk(loo_s[a0:a0 + 48, :]), oo, _NT))
            o_ref[r, b0:b0 + 96, sl] = (x0_s[bufB, r, j, b0:b0 + 96, :] + y).astype(o_ref.dtype)

    left = lane < 64
    mL = jnp.where(left, jnp.uint32(0xFFFFFFFF), jnp.uint32(0))
    mR = jnp.where(left, jnp.uint32(0), jnp.uint32(0xFFFFFFFF))
    key_ok = (jax.lax.broadcasted_iota(jnp.int32, (56, 128), 0) % 8) < _WS
    z8 = jnp.zeros((8, 256), _F32)
    z32 = jnp.zeros((32, 128), _F32)
    z8l = jnp.zeros((8, 128), _F32)

    def softmax_t(s):
        s = jnp.where(key_ok, s, _NEG)
        m = jnp.max(s, axis=0, keepdims=True)
        p = jnp.exp2(s - m)
        l = jnp.sum(p, axis=0, keepdims=True)
        return p, pl.reciprocal(l, approx=False)

    def gather(ref, t0):
        return [jnp.concatenate([ref[bufB, k, r, pl.ds(t0, 8), :] for r in range(_WS)], axis=0)
                for k in range(2)]

    def proj(p, slot):
        ta_ = p * (2 * _WS)
        hA = jnp.concatenate(gather(h_s, ta_), axis=1)
        hB = jnp.concatenate(gather(h_s, ta_ + _WS), axis=1)
        hAB = jnp.concatenate([hA, z8, hB, z8], axis=0).astype(_BF16)
        hBA = jnp.concatenate([hB, z8, hA, z8], axis=0).astype(_BF16)
        r1 = _pk(_dot(_upk(lab_s[...]), hAB, _NT))
        r2 = _pk(_dot(_upk(lba_s[...]), hBA, _NT))
        qe, qo = r1[0:dh], r2[0:dh]
        for t2 in range(2):
            e = qe[(dh // 2) * t2:(dh // 2) * (t2 + 1)]
            o = qo[(dh // 2) * t2:(dh // 2) * (t2 + 1)]
            q_s[slot, 2 * t2] = jnp.concatenate([e & mL, o & mR], axis=0)
            q_s[slot, 2 * t2 + 1] = jnp.concatenate([e & mR, o & mL], axis=0)
        v_s[slot, 0:dh, :] = r1[dh:2 * dh]
        v_s[slot, dh:2 * dh, :] = r2[dh:2 * dh]

    def scores(p, slot):
        ta_ = p * (2 * _WS)
        kA = gather(k_s, ta_)
        kB = gather(k_s, ta_ + _WS)
        out = []
        for t2 in range(2):
            sA = _dot(kA[t2][:, 0:96], _upk(q_s[slot, 2 * t2]), _NN)
            sB = _dot(kB[t2][:, 0:96], _upk(q_s[slot, 2 * t2 + 1]), _NN)
            out.append((sA, sB))
        return out

    def probs(ss, slot):
        for t2 in range(2):
            pA, rA = softmax_t(ss[t2][0])
            pB, rB = softmax_t(ss[t2][1])
            uA = _pk(jnp.concatenate([pA, z8l], axis=0))
            uB = _pk(jnp.concatenate([pB, z8l], axis=0))
            pe, po = [uA & mL, uB & mR], [uA & mR, uB & mL]
            if t2 == 1:
                pe, po = pe[::-1], po[::-1]
            p_s[slot, 2 * t2] = jnp.concatenate(pe, axis=0)
            p_s[slot, 2 * t2 + 1] = jnp.concatenate(po, axis=0)
            r_s[slot, 2 * t2] = jnp.broadcast_to(jnp.where(left, rA, rB), (8, 128))
            r_s[slot, 2 * t2 + 1] = jnp.broadcast_to(jnp.where(left, rB, rA), (8, 128))

    def pv(p, slot):
        ta_ = p * (2 * _WS)
        tb_ = ta_ + _WS
        oe, oo = [], []
        for t2 in range(2):
            v2 = _upk(v_s[slot, dh * t2:dh * (t2 + 1), :])
            oe.append(_dot(v2[0:dh], _upk(p_s[slot, 2 * t2]), _NN) * r_s[slot, 2 * t2, 0:1, :])
            oo.append(_dot(v2[dh:2 * dh], _upk(p_s[slot, 2 * t2 + 1]), _NN)
                      * r_s[slot, 2 * t2 + 1, 0:1, :])
        oeT = jnp.concatenate(oe + [z32], axis=0).astype(_BF16).T.astype(_F32)
        ooT = jnp.concatenate(oo + [z32], axis=0).astype(_BF16).T.astype(_F32)
        for r in range(_WS):
            oe_s[r, pl.ds(ta_, 8), :] = oeT[8 * r:8 * r + 8]
            oo_s[r, pl.ds(ta_, 8), :] = ooT[64 + 8 * r:64 + 8 * r + 8]
        for r in range(_WS):
            oe_s[r, pl.ds(tb_, 8), :] = oeT[64 + 8 * r:64 + 8 * r + 8]
            oo_s[r, pl.ds(tb_, 8), :] = ooT[8 * r:8 * r + 8]

    G = _GROUP
    ngrp = -(-npair // G)
    nslot = 3 * G
    ntile = WP // 128

    def members(g):
        return [(p, p % nslot) for p in range(g * G, min((g + 1) * G, npair))]

    side = {g: [] for g in range(-1, ngrp)}
    for u in range(nunit):
        side[-1 + u // _CUNITS].append(functools.partial(conv_unit, u))
    conv_done = -1 + (nunit - 1) // _CUNITS
    for n in range(nunit):
        r = n // ntile
        ready = -1 + (ntile * r + ntile - 1) // _CUNITS
        g = max(ready + 1, _NORM0 + (n * (ngrp - _NORM0)) // nunit)
        side[min(g, ngrp - 1)].append(functools.partial(norm_unit, r, n % ntile))
    for j in range(ntile):
        ready = min((128 * (j + 1) - 1) // (2 * _WS), npair - 1) // G
        nxt = min((128 * (j + 2) - 1) // (2 * _WS), npair - 1) // G if j + 1 < ntile else ready
        for r in range(_WS):
            g = ready + 1 + (r * (nxt - ready)) // _WS
            if g <= ngrp - 1:
                side[g].append(functools.partial(out_unit, r, j))
    stages = [functools.partial(stage_row, 0, xu_ref, t > 0),
              functools.partial(stage_row, _WS + 1, xd_ref, t < nstrips - 1)]
    stages += [functools.partial(stage_row, r + 1, x_ref, None, r) for r in range(_WS)]
    for n, fn in enumerate(stages):
        g = conv_done + 1 + (n * (ngrp - 1 - conv_done)) // len(stages)
        side[min(g, ngrp - 1)].append(fn)

    def step(g):
        sc = members(g + 1) if g + 1 < ngrp else []
        ss = [scores(p, sl) for p, sl in sc]
        if g >= 0:
            for p, sl in members(g):
                pv(p, sl)
        if g + 2 < ngrp:
            for p, sl in members(g + 2):
                proj(p, sl)
        for s_, (p, sl) in zip(ss, sc):
            probs(s_, sl)
        for fn in side[g]:
            fn()

    for p, sl in members(0):
        proj(p, sl)
    for g in range(-1, ngrp):
        step(g)
    for r in range(_WS):
        out_unit(r, ntile - 1)


@jax.jit
def pallas_standalone__window_attn_davit__vision_kernel(x, dw_pe, w_qkv, w_o):
    B, H, W, C = x.shape
    assert B == 1 and H % _WS == 0 and W % _WS == 0 and W + _WS + 1 <= 520 and C == 192
    nstrips = H // _WS
    WP = 512
    u32 = jnp.uint32
    xt = jnp.transpose(x, (0, 1, 3, 2)).reshape(H, C, W)
    dw = jnp.pad(dw_pe.reshape(9, C), ((0, 7), (0, 256 - C)))
    kern = functools.partial(_kernel, H=H, W=W, C=C, nstrips=nstrips)

    def strip(t):
        return jnp.minimum(t, nstrips - 1)

    out = pl.pallas_call(
        kern,
        grid=(nstrips + 2,),
        in_specs=[
            pl.BlockSpec((_WS, C, WP), lambda t: (strip(t), 0, 0)),
            pl.BlockSpec((1, C, WP), lambda t: (jnp.maximum(strip(t) * _WS - 1, 0), 0, 0)),
            pl.BlockSpec((1, C, WP), lambda t: (jnp.minimum(strip(t) * _WS + _WS, H - 1), 0, 0)),
            pl.BlockSpec((16, 256), lambda t: (0, 0)),
            pl.BlockSpec((C, 3 * C), lambda t: (0, 0)),
            pl.BlockSpec((C, C), lambda t: (0, 0)),
        ],
        out_specs=pl.BlockSpec((_WS, C, WP), lambda t: (jnp.maximum(t - 2, 0), 0, 0)),
        out_shape=jax.ShapeDtypeStruct((H, C, W), x.dtype),
        scratch_shapes=[
            pltpu.VMEM((9, C, 128), _F32),
            pltpu.VMEM((96, 256), u32),
            pltpu.VMEM((96, 256), u32),
            pltpu.VMEM((128, 256), u32),
            pltpu.VMEM((C // 2, 128), u32),
            pltpu.VMEM((C // 2, 128), u32),
            pltpu.VMEM((_WS + 2, C, WP), _F32),
            pltpu.VMEM((2, _WS, WP // 128, C, 128), _F32),
            pltpu.VMEM((2, 2, _WS, WP + 8, 128), _F32),
            pltpu.VMEM((2, 2, _WS, WP + 8, 128), _F32),
            pltpu.VMEM((_WS, WP + 8, 128), _F32),
            pltpu.VMEM((_WS, WP + 8, 128), _F32),
            pltpu.VMEM((3 * _GROUP, 4, 48, 128), u32),
            pltpu.VMEM((3 * _GROUP, 96, 128), u32),
            pltpu.VMEM((3 * _GROUP, 4, 64, 128), u32),
            pltpu.VMEM((3 * _GROUP, 4, 8, 128), _F32),
        ],
        compiler_params=pltpu.CompilerParams(
            dimension_semantics=("arbitrary",),
            vmem_limit_bytes=64 * 1024 * 1024,
        ),
    )(xt, xt, xt, dw, w_qkv, w_o)
    return jnp.transpose(out.reshape(1, H, C, W), (0, 1, 3, 2))
```

```python
import functools

import jax
import jax.numpy as jnp
import jax.experimental.pallas as pl
import jax.experimental.pallas.tpu as pltpu
import numpy as np

_WS = 7
_NH = 4
_NN = (((1,), (0,)), ((), ()))
_NT = (((1,), (1,)), ((), ()))
_F32 = jnp.float32
_BF16 = jnp.bfloat16
_NEG = -1e30
_GROUP = 2
_CUNITS = 2
_NORM0 = 1


def _dot(a, b, dims):
    return jax.lax.dot_general(a, b, dims, preferred_element_type=_F32)


def _xpose(a):
    r, c = a.shape
    rp, cp = -(-r // 128) * 128, -(-c // 128) * 128
    if rp != r:
        a = jnp.concatenate([a, jnp.zeros((rp - r, c), a.dtype)], axis=0)
    if cp != c:
        a = jnp.concatenate([a, jnp.zeros((rp, cp - c), a.dtype)], axis=1)
    return a.T[:c, :r]


def _pk(a):
    return pltpu.bitcast(a.astype(_BF16), jnp.uint32)


def _upk(a):
    return pltpu.bitcast(a, _BF16)


def _kernel(x_ref, xu_ref, xd_ref, dw_ref, wqkv_ref, wo_ref, o_ref,
            wconv_s, lab_s, lba_s, rk_s, loe_s, loo_s,
            xs_s, x0_s, h_s, k_s, oe_s, oo_s, q_s, v_s, p_s, r_s, *, H, W, C, nstrips):
    t = pl.program_id(0)
    dh = C // _NH
    WP = 512
    nwin = W // _WS
    npair = (nwin + 1) // 2
    CH = 48
    nunit = _WS * (C // CH)

    @pl.when(t == 0)
    def _prep():
        def padk(a):
            return jnp.concatenate([a, jnp.zeros((a.shape[0], 256 - C), _F32)], axis=1)
        wT = _xpose(wqkv_ref[...].astype(_F32))
        lab_s[...] = _pk(padk(jnp.concatenate(
            [wT[0:dh], wT[2 * dh:3 * dh], wT[2 * C:2 * C + 2 * dh]], axis=0)))
        lba_s[...] = _pk(padk(jnp.concatenate(
            [wT[dh:2 * dh], wT[3 * dh:4 * dh], wT[2 * C + 2 * dh:3 * C]], axis=0)))
        z = jnp.zeros((128 - 2 * dh, C), _F32)
        kscale = float(dh) ** -0.5 * float(np.log2(np.e))
        k01 = jnp.concatenate([wT[C:C + 2 * dh] * kscale, z], axis=0)
        k23 = jnp.concatenate([wT[C + 2 * dh:2 * C] * kscale, z], axis=0)
        rk_s[...] = _pk(jnp.concatenate([padk(k01).T, padk(k23).T], axis=1))
        wo = wo_ref[...].astype(_F32)
        woe = jnp.concatenate([wo[0:dh], wo[2 * dh:3 * dh], z], axis=0)
        woo = jnp.concatenate([wo[dh:2 * dh], wo[3 * dh:4 * dh], z], axis=0)
        loe_s[...] = _pk(_xpose(woe))
        loo_s[...] = _pk(_xpose(woo))
        dwT = _xpose(dw_ref[...].astype(_F32))
        for k in range(9):
            wk = jnp.broadcast_to(dwT[0:C, k:k + 1], (C, 128))
            wconv_s[k] = wk + 1.0 if k == 4 else wk
        h_s[1, :, :, pl.ds(WP, 8), :] = jnp.zeros((2, _WS, 8, 128), _F32)
        k_s[1, :, :, pl.ds(WP, 8), :] = jnp.zeros((2, _WS, 8, 128), _F32)
        h_s[0] = jnp.zeros(h_s.shape[1:], _F32)
        k_s[0] = jnp.zeros(k_s.shape[1:], _F32)
        xs_s[...] = jnp.zeros(xs_s.shape, _F32)
        x0_s[...] = jnp.zeros(x0_s.shape, _F32)
        oe_s[...] = jnp.zeros(oe_s.shape, _F32)
        oo_s[...] = jnp.zeros(oo_s.shape, _F32)

    def main(bufB, bufA):
        lane = jax.lax.broadcasted_iota(jnp.int32, (1, 128), 1)
        last_ok = lane < (W - (WP - 128))

        def stage_row(dst, ref, ok, src=0):
            v = ref[src].astype(_F32)
            okl = last_ok if ok is None else jnp.logical_and(last_ok, ok)
            lo = v[:, :WP - 128] if ok is None else jnp.where(ok, v[:, :WP - 128], 0.0)
            xs_s[dst, :, :WP - 128] = lo
            xs_s[dst, :, WP - 128:] = jnp.where(okl, v[:, WP - 128:], 0.0)

        def conv_unit(u):
            r = u // (C // CH)
            c0 = (u - r * (C // CH)) * CH
            y = [None, None, None]
            for a in range(3):
                xv = xs_s[r + a, c0:c0 + CH, :]
                for b in range(3):
                    w = wconv_s[3 * a + b, c0:c0 + CH, :]
                    term = xv * jnp.concatenate([w] * (WP // 128), axis=1)
                    y[b] = term if y[b] is None else y[b] + term
            x0 = y[1] + (pltpu.roll(y[0], 1, 1) + pltpu.roll(y[2], WP - 1, 1))
            for j in range(WP // 128):
                x0_s[bufA, r, j, c0:c0 + CH, :] = x0[:, 128 * j:128 * (j + 1)]

        def norm_unit(r, j):
            x0 = x0_s[bufA, r, j]
            mean = jnp.sum(x0, axis=0, keepdims=True) * (1.0 / C)
            ex2 = jnp.sum(x0 * x0, axis=0, keepdims=True) * (1.0 / C)
            rstd = jax.lax.rsqrt(jnp.maximum(ex2 - mean * mean, 0.0) + 1e-5)
            hn = (x0 - mean) * rstd
            hb = jnp.concatenate([hn, jnp.zeros((256 - C, 128), _F32)], axis=0).astype(_BF16).T
            hf = hb.astype(_F32)
            h_s[bufA, 0, r, 128 * j:128 * (j + 1), :] = hf[:, 0:128]
            h_s[bufA, 1, r, 128 * j:128 * (j + 1), :] = hf[:, 128:256]
            kk = _dot(hb, _upk(rk_s[...]), _NN)
            k_s[bufA, 0, r, 128 * j:128 * (j + 1), :] = kk[:, 0:128]
            k_s[bufA, 1, r, 128 * j:128 * (j + 1), :] = kk[:, 128:256]

        def out_unit(r, j):
            sl = slice(128 * j, 128 * (j + 1))
            oe = oe_s[r, sl, :].astype(_BF16)
            oo = oo_s[r, sl, :].astype(_BF16)
            for m in range(2):
                a0, b0 = 48 * m, 96 * m
                y = (_dot(_upk(loe_s[a0:a0 + 48, :]), oe, _NT) + _dot(_upk(loo_s[a0:a0 + 48, :]), oo, _NT))
                o_ref[r, b0:b0 + 96, sl] = (x0_s[bufB, r, j, b0:b0 + 96, :] + y).astype(o_ref.dtype)

        left = lane < 64
        mL = jnp.where(left, jnp.uint32(0xFFFFFFFF), jnp.uint32(0))
        mR = jnp.where(left, jnp.uint32(0), jnp.uint32(0xFFFFFFFF))
        key_ok = (jax.lax.broadcasted_iota(jnp.int32, (56, 128), 0) % 8) < _WS
        z8 = jnp.zeros((8, 256), _F32)
        z32 = jnp.zeros((32, 128), _F32)
        z8l = jnp.zeros((8, 128), _F32)

        def softmax_t(s):
            s = jnp.where(key_ok, s, _NEG)
            m = jnp.max(s, axis=0, keepdims=True)
            p = jnp.exp2(s - m)
            l = jnp.sum(p, axis=0, keepdims=True)
            return p, pl.reciprocal(l, approx=False)

        def gather(ref, t0):
            return [jnp.concatenate([ref[bufB, k, r, pl.ds(t0, 8), :] for r in range(_WS)], axis=0)
                    for k in range(2)]

        def proj(p, slot):
            ta_ = p * (2 * _WS)
            hA = jnp.concatenate(gather(h_s, ta_), axis=1)
            hB = jnp.concatenate(gather(h_s, ta_ + _WS), axis=1)
            hAB = jnp.concatenate([hA, z8, hB, z8], axis=0).astype(_BF16)
            hBA = jnp.concatenate([hB, z8, hA, z8], axis=0).astype(_BF16)
            r1 = _pk(_dot(_upk(lab_s[...]), hAB, _NT))
            r2 = _pk(_dot(_upk(lba_s[...]), hBA, _NT))
            qe, qo = r1[0:dh], r2[0:dh]
            for t2 in range(2):
                e = qe[(dh // 2) * t2:(dh // 2) * (t2 + 1)]
                o = qo[(dh // 2) * t2:(dh // 2) * (t2 + 1)]
                q_s[slot, 2 * t2] = jnp.concatenate([e & mL, o & mR], axis=0)
                q_s[slot, 2 * t2 + 1] = jnp.concatenate([e & mR, o & mL], axis=0)
            v_s[slot, 0:dh, :] = r1[dh:2 * dh]
            v_s[slot, dh:2 * dh, :] = r2[dh:2 * dh]

        def scores(p, slot):
            ta_ = p * (2 * _WS)
            kA = gather(k_s, ta_)
            kB = gather(k_s, ta_ + _WS)
            out = []
            for t2 in range(2):
                sA = _dot(kA[t2][:, 0:96], _upk(q_s[slot, 2 * t2]), _NN)
                sB = _dot(kB[t2][:, 0:96], _upk(q_s[slot, 2 * t2 + 1]), _NN)
                out.append((sA, sB))
            return out

        def probs(ss, slot):
            for t2 in range(2):
                pA, rA = softmax_t(ss[t2][0])
                pB, rB = softmax_t(ss[t2][1])
                uA = _pk(jnp.concatenate([pA, z8l], axis=0))
                uB = _pk(jnp.concatenate([pB, z8l], axis=0))
                pe, po = [uA & mL, uB & mR], [uA & mR, uB & mL]
                if t2 == 1:
                    pe, po = pe[::-1], po[::-1]
                p_s[slot, 2 * t2] = jnp.concatenate(pe, axis=0)
                p_s[slot, 2 * t2 + 1] = jnp.concatenate(po, axis=0)
                r_s[slot, 2 * t2] = jnp.broadcast_to(jnp.where(left, rA, rB), (8, 128))
                r_s[slot, 2 * t2 + 1] = jnp.broadcast_to(jnp.where(left, rB, rA), (8, 128))

        def pv(p, slot):
            ta_ = p * (2 * _WS)
            tb_ = ta_ + _WS
            oe, oo = [], []
            for t2 in range(2):
                v2 = _upk(v_s[slot, dh * t2:dh * (t2 + 1), :])
                oe.append(_dot(v2[0:dh], _upk(p_s[slot, 2 * t2]), _NN) * r_s[slot, 2 * t2, 0:1, :])
                oo.append(_dot(v2[dh:2 * dh], _upk(p_s[slot, 2 * t2 + 1]), _NN)
                          * r_s[slot, 2 * t2 + 1, 0:1, :])
            oeT = jnp.concatenate(oe + [z32], axis=0).astype(_BF16).T.astype(_F32)
            ooT = jnp.concatenate(oo + [z32], axis=0).astype(_BF16).T.astype(_F32)
            for r in range(_WS):
                oe_s[r, pl.ds(ta_, 8), :] = oeT[8 * r:8 * r + 8]
                oo_s[r, pl.ds(ta_, 8), :] = ooT[64 + 8 * r:64 + 8 * r + 8]
            for r in range(_WS):
                oe_s[r, pl.ds(tb_, 8), :] = oeT[64 + 8 * r:64 + 8 * r + 8]
                oo_s[r, pl.ds(tb_, 8), :] = ooT[8 * r:8 * r + 8]

        G = _GROUP
        ngrp = -(-npair // G)
        nslot = 3 * G
        ntile = WP // 128

        def members(g):
            return [(p, p % nslot) for p in range(g * G, min((g + 1) * G, npair))]

        side = {g: [] for g in range(-1, ngrp)}
        for u in range(nunit):
            side[-1 + u // _CUNITS].append(functools.partial(conv_unit, u))
        conv_done = -1 + (nunit - 1) // _CUNITS
        for n in range(nunit):
            r = n // ntile
            ready = -1 + (ntile * r + ntile - 1) // _CUNITS
            g = max(ready + 1, _NORM0 + (n * (ngrp - _NORM0)) // nunit)
            side[min(g, ngrp - 1)].append(functools.partial(norm_unit, r, n % ntile))
        for j in range(ntile):
            ready = min((128 * (j + 1) - 1) // (2 * _WS), npair - 1) // G
            nxt = min((128 * (j + 2) - 1) // (2 * _WS), npair - 1) // G if j + 1 < ntile else ready
            for r in range(_WS):
                g = ready + 1 + (r * (nxt - ready)) // _WS
                if g <= ngrp - 1:
                    side[g].append(functools.partial(out_unit, r, j))
        stages = [functools.partial(stage_row, 0, xu_ref, t > 0),
                  functools.partial(stage_row, _WS + 1, xd_ref, t < nstrips - 1)]
        stages += [functools.partial(stage_row, r + 1, x_ref, None, r) for r in range(_WS)]
        for n, fn in enumerate(stages):
            g = conv_done + 1 + (n * (ngrp - 1 - conv_done)) // len(stages)
            side[min(g, ngrp - 1)].append(fn)

        def step(g):
            sc = members(g + 1) if g + 1 < ngrp else []
            ss = [scores(p, sl) for p, sl in sc]
            if g >= 0:
                for p, sl in members(g):
                    pv(p, sl)
            if g + 2 < ngrp:
                for p, sl in members(g + 2):
                    proj(p, sl)
            for s_, (p, sl) in zip(ss, sc):
                probs(s_, sl)
            for fn in side[g]:
                fn()

        for p, sl in members(0):
            proj(p, sl)
        for g in range(-1, ngrp):
            step(g)
        for r in range(_WS):
            out_unit(r, ntile - 1)

    parity = jax.lax.rem(t, 2)

    @pl.when(parity == 0)
    def _even():
        main(0, 1)

    @pl.when(parity == 1)
    def _odd():
        main(1, 0)


@jax.jit
def pallas_standalone__window_attn_davit__vision_kernel(x, dw_pe, w_qkv, w_o):
    B, H, W, C = x.shape
    assert B == 1 and H % _WS == 0 and W % _WS == 0 and W + _WS + 1 <= 520 and C == 192
    nstrips = H // _WS
    WP = 512
    u32 = jnp.uint32
    xt = jnp.transpose(x, (0, 1, 3, 2)).reshape(H, C, W)
    dw = jnp.pad(dw_pe.reshape(9, C), ((0, 7), (0, 256 - C)))
    kern = functools.partial(_kernel, H=H, W=W, C=C, nstrips=nstrips)

    def strip(t):
        return jnp.minimum(t, nstrips - 1)

    out = pl.pallas_call(
        kern,
        grid=(nstrips + 2,),
        in_specs=[
            pl.BlockSpec((_WS, C, WP), lambda t: (strip(t), 0, 0)),
            pl.BlockSpec((1, C, WP), lambda t: (jnp.maximum(strip(t) * _WS - 1, 0), 0, 0)),
            pl.BlockSpec((1, C, WP), lambda t: (jnp.minimum(strip(t) * _WS + _WS, H - 1), 0, 0)),
            pl.BlockSpec((16, 256), lambda t: (0, 0)),
            pl.BlockSpec((C, 3 * C), lambda t: (0, 0)),
            pl.BlockSpec((C, C), lambda t: (0, 0)),
        ],
        out_specs=pl.BlockSpec((_WS, C, WP), lambda t: (jnp.maximum(t - 2, 0), 0, 0)),
        out_shape=jax.ShapeDtypeStruct((H, C, W), x.dtype),
        scratch_shapes=[
            pltpu.VMEM((9, C, 128), _F32),
            pltpu.VMEM((96, 256), u32),
            pltpu.VMEM((96, 256), u32),
            pltpu.VMEM((128, 256), u32),
            pltpu.VMEM((C // 2, 128), u32),
            pltpu.VMEM((C // 2, 128), u32),
            pltpu.VMEM((_WS + 2, C, WP), _F32),
            pltpu.VMEM((2, _WS, WP // 128, C, 128), _F32),
            pltpu.VMEM((2, 2, _WS, WP + 8, 128), _F32),
            pltpu.VMEM((2, 2, _WS, WP + 8, 128), _F32),
            pltpu.VMEM((_WS, WP + 8, 128), _F32),
            pltpu.VMEM((_WS, WP + 8, 128), _F32),
            pltpu.VMEM((3 * _GROUP, 4, 48, 128), u32),
            pltpu.VMEM((3 * _GROUP, 96, 128), u32),
            pltpu.VMEM((3 * _GROUP, 4, 64, 128), u32),
            pltpu.VMEM((3 * _GROUP, 4, 8, 128), _F32),
        ],
        compiler_params=pltpu.CompilerParams(
            dimension_semantics=("arbitrary",),
            vmem_limit_bytes=64 * 1024 * 1024,
        ),
    )(xt, xt, xt, dw, w_qkv, w_o)
    return jnp.transpose(out.reshape(1, H, C, W), (0, 1, 3, 2))
```

```python
import functools

import jax
import jax.numpy as jnp
import jax.experimental.pallas as pl
import jax.experimental.pallas.tpu as pltpu
import numpy as np

_WS = 7
_NH = 4
_NN = (((1,), (0,)), ((), ()))
_NT = (((1,), (1,)), ((), ()))
_F32 = jnp.float32
_BF16 = jnp.bfloat16
_NEG = -1e30
_GROUP = 2
_CUNITS = 2
_NORM0 = 1


def _dot(a, b, dims):
    return jax.lax.dot_general(a, b, dims, preferred_element_type=_F32)


def _xpose(a):
    r, c = a.shape
    rp, cp = -(-r // 128) * 128, -(-c // 128) * 128
    if rp != r:
        a = jnp.concatenate([a, jnp.zeros((rp - r, c), a.dtype)], axis=0)
    if cp != c:
        a = jnp.concatenate([a, jnp.zeros((rp, cp - c), a.dtype)], axis=1)
    return a.T[:c, :r]


def _pk(a):
    return pltpu.bitcast(a.astype(_BF16), jnp.uint32)


def _upk(a):
    return pltpu.bitcast(a, _BF16)


def _kernel(x_ref, xu_ref, xd_ref, dw_ref, wqkv_ref, wo_ref, o_ref,
            wconv_s, lab_s, lba_s, rk_s, loe_s, loo_s,
            xs_s, x0_s, h_s, k_s, oe_s, oo_s, *, H, W, C, nstrips):
    t = pl.program_id(0)
    dh = C // _NH
    WP = 512
    nwin = W // _WS
    npair = (nwin + 1) // 2
    CH = 48
    nunit = _WS * (C // CH)

    @pl.when(t == 0)
    def _prep():
        def padk(a):
            return jnp.concatenate([a, jnp.zeros((a.shape[0], 256 - C), _F32)], axis=1)
        wT = _xpose(wqkv_ref[...].astype(_F32))
        lab_s[...] = _pk(padk(jnp.concatenate(
            [wT[0:dh], wT[2 * dh:3 * dh], wT[2 * C:2 * C + 2 * dh]], axis=0)))
        lba_s[...] = _pk(padk(jnp.concatenate(
            [wT[dh:2 * dh], wT[3 * dh:4 * dh], wT[2 * C + 2 * dh:3 * C]], axis=0)))
        z = jnp.zeros((128 - 2 * dh, C), _F32)
        kscale = float(dh) ** -0.5 * float(np.log2(np.e))
        k01 = jnp.concatenate([wT[C:C + 2 * dh] * kscale, z], axis=0)
        k23 = jnp.concatenate([wT[C + 2 * dh:2 * C] * kscale, z], axis=0)
        rk_s[...] = _pk(jnp.concatenate([padk(k01).T, padk(k23).T], axis=1))
        wo = wo_ref[...].astype(_F32)
        woe = jnp.concatenate([wo[0:dh], wo[2 * dh:3 * dh], z], axis=0)
        woo = jnp.concatenate([wo[dh:2 * dh], wo[3 * dh:4 * dh], z], axis=0)
        loe_s[...] = _pk(_xpose(woe))
        loo_s[...] = _pk(_xpose(woo))
        dwT = _xpose(dw_ref[...].astype(_F32))
        for k in range(9):
            wk = jnp.broadcast_to(dwT[0:C, k:k + 1], (C, 128))
            wconv_s[k] = wk + 1.0 if k == 4 else wk
        h_s[1, :, :, pl.ds(WP, 8), :] = jnp.zeros((2, _WS, 8, 128), _F32)
        k_s[1, :, :, pl.ds(WP, 8), :] = jnp.zeros((2, _WS, 8, 128), _F32)
        h_s[0] = jnp.zeros(h_s.shape[1:], _F32)
        k_s[0] = jnp.zeros(k_s.shape[1:], _F32)
        xs_s[...] = jnp.zeros(xs_s.shape, _F32)
        x0_s[...] = jnp.zeros(x0_s.shape, _F32)
        oe_s[...] = jnp.zeros(oe_s.shape, _F32)
        oo_s[...] = jnp.zeros(oo_s.shape, _F32)

    def main(bufB, bufA):
        lane = jax.lax.broadcasted_iota(jnp.int32, (1, 128), 1)
        last_ok = lane < (W - (WP - 128))

        def stage_row(dst, ref, ok, src=0):
            v = ref[src].astype(_F32)
            okl = last_ok if ok is None else jnp.logical_and(last_ok, ok)
            lo = v[:, :WP - 128] if ok is None else jnp.where(ok, v[:, :WP - 128], 0.0)
            xs_s[dst, :, :WP - 128] = lo
            xs_s[dst, :, WP - 128:] = jnp.where(okl, v[:, WP - 128:], 0.0)

        def conv_unit(u):
            r = u // (C // CH)
            c0 = (u - r * (C // CH)) * CH
            y = [None, None, None]
            for a in range(3):
                xv = xs_s[r + a, c0:c0 + CH, :]
                for b in range(3):
                    w = wconv_s[3 * a + b, c0:c0 + CH, :]
                    term = xv * jnp.concatenate([w] * (WP // 128), axis=1)
                    y[b] = term if y[b] is None else y[b] + term
            x0 = y[1] + (pltpu.roll(y[0], 1, 1) + pltpu.roll(y[2], WP - 1, 1))
            for j in range(WP // 128):
                x0_s[bufA, r, j, c0:c0 + CH, :] = x0[:, 128 * j:128 * (j + 1)]

        def norm_unit(r, j):
            x0 = x0_s[bufA, r, j]
            mean = jnp.sum(x0, axis=0, keepdims=True) * (1.0 / C)
            ex2 = jnp.sum(x0 * x0, axis=0, keepdims=True) * (1.0 / C)
            rstd = jax.lax.rsqrt(jnp.maximum(ex2 - mean * mean, 0.0) + 1e-5)
            hn = (x0 - mean) * rstd
            hb = jnp.concatenate([hn, jnp.zeros((256 - C, 128), _F32)], axis=0).astype(_BF16).T
            hf = hb.astype(_F32)
            h_s[bufA, 0, r, 128 * j:128 * (j + 1), :] = hf[:, 0:128]
            h_s[bufA, 1, r, 128 * j:128 * (j + 1), :] = hf[:, 128:256]
            kk = _dot(hb, _upk(rk_s[...]), _NN)
            k_s[bufA, 0, r, 128 * j:128 * (j + 1), :] = kk[:, 0:128]
            k_s[bufA, 1, r, 128 * j:128 * (j + 1), :] = kk[:, 128:256]

        def out_unit(r, j):
            sl = slice(128 * j, 128 * (j + 1))
            oe = oe_s[r, sl, :].astype(_BF16)
            oo = oo_s[r, sl, :].astype(_BF16)
            for m in range(2):
                a0, b0 = 48 * m, 96 * m
                y = (_dot(_upk(loe_s[a0:a0 + 48, :]), oe, _NT) + _dot(_upk(loo_s[a0:a0 + 48, :]), oo, _NT))
                o_ref[r, b0:b0 + 96, sl] = (x0_s[bufB, r, j, b0:b0 + 96, :] + y).astype(o_ref.dtype)

        left = lane < 64
        qv, pr = {}, {}

        def selL(a):
            return jnp.where(left, a, 0.0)

        def selR(a):
            return jnp.where(left, 0.0, a)

        key_ok = (jax.lax.broadcasted_iota(jnp.int32, (56, 128), 0) % 8) < _WS
        z8 = jnp.zeros((8, 256), _F32)
        z32 = jnp.zeros((32, 128), _F32)
        z8l = jnp.zeros((8, 128), _F32)

        def softmax_t(s):
            s = jnp.where(key_ok, s, _NEG)
            m = jnp.max(s, axis=0, keepdims=True)
            p = jnp.exp2(s - m)
            l = jnp.sum(p, axis=0, keepdims=True)
            return p, pl.reciprocal(l, approx=False)

        def gather(ref, t0):
            return [jnp.concatenate([ref[bufB, k, r, pl.ds(t0, 8), :] for r in range(_WS)], axis=0)
                    for k in range(2)]

        def proj(p, slot):
            ta_ = p * (2 * _WS)
            hA = jnp.concatenate(gather(h_s, ta_), axis=1)
            hB = jnp.concatenate(gather(h_s, ta_ + _WS), axis=1)
            hAB = jnp.concatenate([hA, z8, hB, z8], axis=0).astype(_BF16)
            hBA = jnp.concatenate([hB, z8, hA, z8], axis=0).astype(_BF16)
            r1 = _dot(_upk(lab_s[...]), hAB, _NT)
            r2 = _dot(_upk(lba_s[...]), hBA, _NT)
            qs = []
            for t2 in range(2):
                e = r1[dh * t2:dh * (t2 + 1)]
                o = r2[dh * t2:dh * (t2 + 1)]
                qs.append(jnp.concatenate([selL(e), selR(o)], axis=0).astype(_BF16))
                qs.append(jnp.concatenate([selR(e), selL(o)], axis=0).astype(_BF16))
            qv[p] = (qs, (r1[2 * dh:4 * dh].astype(_BF16),
                          r2[2 * dh:4 * dh].astype(_BF16)))

        def scores(p, slot):
            ta_ = p * (2 * _WS)
            kA = gather(k_s, ta_)
            kB = gather(k_s, ta_ + _WS)
            out = []
            for t2 in range(2):
                sA = _dot(kA[t2][:, 0:96], qv[p][0][2 * t2], _NN)
                sB = _dot(kB[t2][:, 0:96], qv[p][0][2 * t2 + 1], _NN)
                out.append((sA, sB))
            return out

        def probs(ss, slot):
            out = []
            for t2 in range(2):
                pA, rA = softmax_t(ss[t2][0])
                pB, rB = softmax_t(ss[t2][1])
                pe, po = [selL(pA), z8l, selR(pB), z8l], [selR(pA), z8l, selL(pB), z8l]
                if t2 == 1:
                    pe, po = pe[2:] + pe[:2], po[2:] + po[:2]
                out.append((jnp.concatenate(pe, axis=0).astype(_BF16),
                            jnp.concatenate(po, axis=0).astype(_BF16),
                            jnp.where(left, rA, rB), jnp.where(left, rB, rA)))
            pr[slot] = out

        def pv(p, slot):
            ta_ = p * (2 * _WS)
            tb_ = ta_ + _WS
            oe, oo = [], []
            for t2 in range(2):
                v2 = qv[p][1][t2]
                pe, po, re_, ro_ = pr[p][t2]
                oe.append(_dot(v2[0:dh], pe, _NN) * re_)
                oo.append(_dot(v2[dh:2 * dh], po, _NN) * ro_)
            oeT = jnp.concatenate(oe + [z32], axis=0).astype(_BF16).T.astype(_F32)
            ooT = jnp.concatenate(oo + [z32], axis=0).astype(_BF16).T.astype(_F32)
            for r in range(_WS):
                oe_s[r, pl.ds(ta_, 8), :] = oeT[8 * r:8 * r + 8]
                oo_s[r, pl.ds(ta_, 8), :] = ooT[64 + 8 * r:64 + 8 * r + 8]
            for r in range(_WS):
                oe_s[r, pl.ds(tb_, 8), :] = oeT[64 + 8 * r:64 + 8 * r + 8]
                oo_s[r, pl.ds(tb_, 8), :] = ooT[8 * r:8 * r + 8]

        G = _GROUP
        ngrp = -(-npair // G)
        nslot = 3 * G
        ntile = WP // 128

        def members(g):
            return [(p, p) for p in range(g * G, min((g + 1) * G, npair))]

        side = {g: [] for g in range(-1, ngrp)}
        for u in range(nunit):
            side[-1 + u // _CUNITS].append(functools.partial(conv_unit, u))
        conv_done = -1 + (nunit - 1) // _CUNITS
        for n in range(nunit):
            r = n // ntile
            ready = -1 + (ntile * r + ntile - 1) // _CUNITS
            g = max(ready + 1, _NORM0 + (n * (ngrp - _NORM0)) // nunit)
            side[min(g, ngrp - 1)].append(functools.partial(norm_unit, r, n % ntile))
        for j in range(ntile):
            ready = min((128 * (j + 1) - 1) // (2 * _WS), npair - 1) // G
            nxt = min((128 * (j + 2) - 1) // (2 * _WS), npair - 1) // G if j + 1 < ntile else ready
            for r in range(_WS):
                g = ready + 1 + (r * (nxt - ready)) // _WS
                if g <= ngrp - 1:
                    side[g].append(functools.partial(out_unit, r, j))
        stages = [functools.partial(stage_row, 0, xu_ref, t > 0),
                  functools.partial(stage_row, _WS + 1, xd_ref, t < nstrips - 1)]
        stages += [functools.partial(stage_row, r + 1, x_ref, None, r) for r in range(_WS)]
        for n, fn in enumerate(stages):
            g = conv_done + 1 + (n * (ngrp - 1 - conv_done)) // len(stages)
            side[min(g, ngrp - 1)].append(fn)

        def step(g):
            sc = members(g + 1) if g + 1 < ngrp else []
            ss = [scores(p, sl) for p, sl in sc]
            if g >= 0:
                for p, sl in members(g):
                    pv(p, sl)
            if g + 2 < ngrp:
                for p, sl in members(g + 2):
                    proj(p, sl)
            for s_, (p, sl) in zip(ss, sc):
                probs(s_, sl)
            for fn in side[g]:
                fn()

        for p, sl in members(0):
            proj(p, sl)
        for g in range(-1, ngrp):
            step(g)
        for r in range(_WS):
            out_unit(r, ntile - 1)

    parity = jax.lax.rem(t, 2)

    @pl.when(parity == 0)
    def _even():
        main(0, 1)

    @pl.when(parity == 1)
    def _odd():
        main(1, 0)


@jax.jit
def pallas_standalone__window_attn_davit__vision_kernel(x, dw_pe, w_qkv, w_o):
    B, H, W, C = x.shape
    assert B == 1 and H % _WS == 0 and W % _WS == 0 and W + _WS + 1 <= 520 and C == 192
    nstrips = H // _WS
    WP = 512
    u32 = jnp.uint32
    xt = jnp.transpose(x, (0, 1, 3, 2)).reshape(H, C, W)
    dw = jnp.pad(dw_pe.reshape(9, C), ((0, 7), (0, 256 - C)))
    kern = functools.partial(_kernel, H=H, W=W, C=C, nstrips=nstrips)

    def strip(t):
        return jnp.minimum(t, nstrips - 1)

    out = pl.pallas_call(
        kern,
        grid=(nstrips + 2,),
        in_specs=[
            pl.BlockSpec((_WS, C, WP), lambda t: (strip(t), 0, 0)),
            pl.BlockSpec((1, C, WP), lambda t: (jnp.maximum(strip(t) * _WS - 1, 0), 0, 0)),
            pl.BlockSpec((1, C, WP), lambda t: (jnp.minimum(strip(t) * _WS + _WS, H - 1), 0, 0)),
            pl.BlockSpec((16, 256), lambda t: (0, 0)),
            pl.BlockSpec((C, 3 * C), lambda t: (0, 0)),
            pl.BlockSpec((C, C), lambda t: (0, 0)),
        ],
        out_specs=pl.BlockSpec((_WS, C, WP), lambda t: (jnp.maximum(t - 2, 0), 0, 0)),
        out_shape=jax.ShapeDtypeStruct((H, C, W), x.dtype),
        scratch_shapes=[
            pltpu.VMEM((9, C, 128), _F32),
            pltpu.VMEM((96, 256), u32),
            pltpu.VMEM((96, 256), u32),
            pltpu.VMEM((128, 256), u32),
            pltpu.VMEM((C // 2, 128), u32),
            pltpu.VMEM((C // 2, 128), u32),
            pltpu.VMEM((_WS + 2, C, WP), _F32),
            pltpu.VMEM((2, _WS, WP // 128, C, 128), _F32),
            pltpu.VMEM((2, 2, _WS, WP + 8, 128), _F32),
            pltpu.VMEM((2, 2, _WS, WP + 8, 128), _F32),
            pltpu.VMEM((_WS, WP + 8, 128), _F32),
            pltpu.VMEM((_WS, WP + 8, 128), _F32),
        ],
        compiler_params=pltpu.CompilerParams(
            dimension_semantics=("arbitrary",),
            vmem_limit_bytes=64 * 1024 * 1024,
        ),
    )(xt, xt, xt, dw, w_qkv, w_o)
    return jnp.transpose(out.reshape(1, H, C, W), (0, 1, 3, 2))
```

```python
import functools

import jax
import jax.numpy as jnp
import jax.experimental.pallas as pl
import jax.experimental.pallas.tpu as pltpu
import numpy as np

_WS = 7
_NH = 4
_NN = (((1,), (0,)), ((), ()))
_NT = (((1,), (1,)), ((), ()))
_F32 = jnp.float32
_BF16 = jnp.bfloat16
_NEG = -1e30
_GROUP = 2
_CSPAN = 14
_NLAG = 1
_ORDER = "SVPRX"
_NORM0 = 1


def _dot(a, b, dims):
    return jax.lax.dot_general(a, b, dims, preferred_element_type=_F32)


def _xpose(a):
    r, c = a.shape
    rp, cp = -(-r // 128) * 128, -(-c // 128) * 128
    if rp != r:
        a = jnp.concatenate([a, jnp.zeros((rp - r, c), a.dtype)], axis=0)
    if cp != c:
        a = jnp.concatenate([a, jnp.zeros((rp, cp - c), a.dtype)], axis=1)
    return a.T[:c, :r]


def _pk(a):
    return pltpu.bitcast(a.astype(_BF16), jnp.uint32)


def _upk(a):
    return pltpu.bitcast(a, _BF16)


def _kernel(x_ref, xu_ref, xd_ref, dw_ref, wqkv_ref, wo_ref, o_ref,
            wconv_s, lab_s, lba_s, rk_s, loe_s, loo_s,
            xs_s, x0_s, h_s, k_s, oe_s, oo_s, *, H, W, C, nstrips):
    t = pl.program_id(0)
    dh = C // _NH
    WP = 512
    nwin = W // _WS
    npair = (nwin + 1) // 2
    CH = 48
    nunit = _WS * (C // CH)

    @pl.when(t == 0)
    def _prep():
        def padk(a):
            return jnp.concatenate([a, jnp.zeros((a.shape[0], 256 - C), _F32)], axis=1)
        wT = _xpose(wqkv_ref[...].astype(_F32))
        lab_s[...] = _pk(padk(jnp.concatenate(
            [wT[0:dh], wT[2 * dh:3 * dh], wT[2 * C:2 * C + 2 * dh]], axis=0)))
        lba_s[...] = _pk(padk(jnp.concatenate(
            [wT[dh:2 * dh], wT[3 * dh:4 * dh], wT[2 * C + 2 * dh:3 * C]], axis=0)))
        z = jnp.zeros((128 - 2 * dh, C), _F32)
        kscale = float(dh) ** -0.5 * float(np.log2(np.e))
        k01 = jnp.concatenate([wT[C:C + 2 * dh] * kscale, z], axis=0)
        k23 = jnp.concatenate([wT[C + 2 * dh:2 * C] * kscale, z], axis=0)
        rk_s[...] = _pk(jnp.concatenate([padk(k01).T, padk(k23).T], axis=1))
        wo = wo_ref[...].astype(_F32)
        woe = jnp.concatenate([wo[0:dh], wo[2 * dh:3 * dh], z], axis=0)
        woo = jnp.concatenate([wo[dh:2 * dh], wo[3 * dh:4 * dh], z], axis=0)
        loe_s[...] = _pk(_xpose(woe))
        loo_s[...] = _pk(_xpose(woo))
        dwT = _xpose(dw_ref[...].astype(_F32))
        for k in range(9):
            wk = jnp.broadcast_to(dwT[0:C, k:k + 1], (C, 128))
            wconv_s[k] = wk + 1.0 if k == 4 else wk
        h_s[:, :, :, pl.ds(WP, 8), :] = jnp.zeros((2, 2, _WS, 8, 128), _F32)
        k_s[:, :, :, pl.ds(WP, 8), :] = jnp.zeros((2, 2, _WS, 8, 128), _F32)

    def main(bufB, bufA, do_att=True, do_conv=True, do_stage=True):
        lane = jax.lax.broadcasted_iota(jnp.int32, (1, 128), 1)
        last_ok = lane < (W - (WP - 128))

        def stage_row(dst, ref, ok, src=0):
            v = ref[src].astype(_F32)
            okl = last_ok if ok is None else jnp.logical_and(last_ok, ok)
            lo = v[:, :WP - 128] if ok is None else jnp.where(ok, v[:, :WP - 128], 0.0)
            xs_s[dst, :, :WP - 128] = lo
            xs_s[dst, :, WP - 128:] = jnp.where(okl, v[:, WP - 128:], 0.0)

        def conv_unit(u):
            r = u // (C // CH)
            c0 = (u - r * (C // CH)) * CH
            y = [None, None, None]
            for a in range(3):
                xv = xs_s[r + a, c0:c0 + CH, :]
                for b in range(3):
                    w = wconv_s[3 * a + b, c0:c0 + CH, :]
                    term = xv * jnp.concatenate([w] * (WP // 128), axis=1)
                    y[b] = term if y[b] is None else y[b] + term
            x0 = y[1] + (pltpu.roll(y[0], 1, 1) + pltpu.roll(y[2], WP - 1, 1))
            for j in range(WP // 128):
                x0_s[bufA, r, j, c0:c0 + CH, :] = x0[:, 128 * j:128 * (j + 1)]

        def norm_unit(r, j):
            x0 = x0_s[bufA, r, j]
            mean = jnp.sum(x0, axis=0, keepdims=True) * (1.0 / C)
            ex2 = jnp.sum(x0 * x0, axis=0, keepdims=True) * (1.0 / C)
            rstd = jax.lax.rsqrt(jnp.maximum(ex2 - mean * mean, 0.0) + 1e-5)
            hn = (x0 - mean) * rstd
            hb = jnp.concatenate([hn, jnp.zeros((256 - C, 128), _F32)], axis=0).astype(_BF16).T
            hf = hb.astype(_F32)
            h_s[bufA, 0, r, 128 * j:128 * (j + 1), :] = hf[:, 0:128]
            h_s[bufA, 1, r, 128 * j:128 * (j + 1), :] = hf[:, 128:256]
            kk = _dot(hb, _upk(rk_s[...]), _NN)
            k_s[bufA, 0, r, 128 * j:128 * (j + 1), :] = kk[:, 0:128]
            k_s[bufA, 1, r, 128 * j:128 * (j + 1), :] = kk[:, 128:256]

        def out_unit(r, j):
            sl = slice(128 * j, 128 * (j + 1))
            oe = oe_s[r, sl, :].astype(_BF16)
            oo = oo_s[r, sl, :].astype(_BF16)
            for m in range(2):
                a0, b0 = 48 * m, 96 * m
                y = (_dot(_upk(loe_s[a0:a0 + 48, :]), oe, _NT) + _dot(_upk(loo_s[a0:a0 + 48, :]), oo, _NT))
                o_ref[r, b0:b0 + 96, sl] = (x0_s[bufB, r, j, b0:b0 + 96, :] + y).astype(o_ref.dtype)

        left = lane < 64
        qv, pr = {}, {}

        def selL(a):
            return jnp.where(left, a, 0.0)

        def selR(a):
            return jnp.where(left, 0.0, a)

        key_ok = (jax.lax.broadcasted_iota(jnp.int32, (56, 128), 0) % 8) < _WS
        z8 = jnp.zeros((8, 256), _F32)
        z32 = jnp.zeros((32, 128), _F32)
        z8l = jnp.zeros((8, 128), _F32)

        def softmax_t(s):
            s = jnp.where(key_ok, s, _NEG)
            m = jnp.max(s, axis=0, keepdims=True)
            p = jnp.exp2(s - m)
            l = jnp.sum(p, axis=0, keepdims=True)
            return p, pl.reciprocal(l, approx=False)

        def gather(ref, t0):
            return [jnp.concatenate([ref[bufB, k, r, pl.ds(t0, 8), :] for r in range(_WS)], axis=0)
                    for k in range(2)]

        def proj(p, slot):
            ta_ = p * (2 * _WS)
            hA = jnp.concatenate(gather(h_s, ta_), axis=1)
            hB = jnp.concatenate(gather(h_s, ta_ + _WS), axis=1)
            hAB = jnp.concatenate([hA, z8, hB, z8], axis=0).astype(_BF16)
            hBA = jnp.concatenate([hB, z8, hA, z8], axis=0).astype(_BF16)
            r1 = _dot(_upk(lab_s[...]), hAB, _NT)
            r2 = _dot(_upk(lba_s[...]), hBA, _NT)
            qs = []
            for t2 in range(2):
                e = r1[dh * t2:dh * (t2 + 1)]
                o = r2[dh * t2:dh * (t2 + 1)]
                qs.append(jnp.concatenate([selL(e), selR(o)], axis=0).astype(_BF16))
                qs.append(jnp.concatenate([selR(e), selL(o)], axis=0).astype(_BF16))
            qv[p] = (qs, (r1[2 * dh:4 * dh].astype(_BF16),
                          r2[2 * dh:4 * dh].astype(_BF16)))

        def scores(p, slot):
            ta_ = p * (2 * _WS)
            kA = gather(k_s, ta_)
            kB = gather(k_s, ta_ + _WS)
            out = []
            for t2 in range(2):
                sA = _dot(kA[t2][:, 0:96], qv[p][0][2 * t2], _NN)
                sB = _dot(kB[t2][:, 0:96], qv[p][0][2 * t2 + 1], _NN)
                out.append((sA, sB))
            return out

        def probs(ss, slot):
            out = []
            for t2 in range(2):
                pA, rA = softmax_t(ss[t2][0])
                pB, rB = softmax_t(ss[t2][1])
                pe, po = [selL(pA), z8l, selR(pB), z8l], [selR(pA), z8l, selL(pB), z8l]
                if t2 == 1:
                    pe, po = pe[2:] + pe[:2], po[2:] + po[:2]
                out.append((jnp.concatenate(pe, axis=0).astype(_BF16),
                            jnp.concatenate(po, axis=0).astype(_BF16),
                            jnp.where(left, rA, rB), jnp.where(left, rB, rA)))
            pr[slot] = out

        def pv(p, slot):
            ta_ = p * (2 * _WS)
            tb_ = ta_ + _WS
            oe, oo = [], []
            for t2 in range(2):
                v2 = qv[p][1][t2]
                pe, po, re_, ro_ = pr[p][t2]
                oe.append(_dot(v2[0:dh], pe, _NN) * re_)
                oo.append(_dot(v2[dh:2 * dh], po, _NN) * ro_)
            oeT = jnp.concatenate(oe + [z32], axis=0).astype(_BF16).T.astype(_F32)
            ooT = jnp.concatenate(oo + [z32], axis=0).astype(_BF16).T.astype(_F32)
            for r in range(_WS):
                oe_s[r, pl.ds(ta_, 8), :] = oeT[8 * r:8 * r + 8]
                oo_s[r, pl.ds(ta_, 8), :] = ooT[64 + 8 * r:64 + 8 * r + 8]
            for r in range(_WS):
                oe_s[r, pl.ds(tb_, 8), :] = oeT[64 + 8 * r:64 + 8 * r + 8]
                oo_s[r, pl.ds(tb_, 8), :] = ooT[8 * r:8 * r + 8]

        G = _GROUP
        ngrp = -(-npair // G)
        nslot = 3 * G
        ntile = WP // 128

        def members(g):
            return [(p, p) for p in range(g * G, min((g + 1) * G, npair))]

        side = {g: [] for g in range(-1, ngrp)}
        conv_at = [-1 + (u * _CSPAN) // nunit for u in range(nunit)]
        conv_done = conv_at[-1] if do_conv else -2
        for u in range(nunit if do_conv else 0):
            side[conv_at[u]].append(functools.partial(conv_unit, u))
        for n in range(nunit if do_conv else 0):
            r = n // ntile
            ready = conv_at[ntile * r + ntile - 1]
            g = max(ready + _NLAG, _NORM0 + (n * (ngrp - _NORM0)) // nunit)
            side[min(g, ngrp - 1)].append(functools.partial(norm_unit, r, n % ntile))
        for j in range(ntile if do_att else 0):
            ready = min((128 * (j + 1) - 1) // (2 * _WS), npair - 1) // G
            nxt = min((128 * (j + 2) - 1) // (2 * _WS), npair - 1) // G if j + 1 < ntile else ready
            for r in range(_WS):
                g = ready + 1 + (r * (nxt - ready)) // _WS
                if g <= ngrp - 1:
                    side[g].append(functools.partial(out_unit, r, j))
        stages = [functools.partial(stage_row, 0, xu_ref, t > 0),
                  functools.partial(stage_row, _WS + 1, xd_ref, t < nstrips - 1)]
        stages += [functools.partial(stage_row, r + 1, x_ref, None, r) for r in range(_WS)]
        for n, fn in enumerate(stages if do_stage else []):
            g = conv_done + 1 + (n * (ngrp - 1 - conv_done)) // len(stages)
            side[min(g, ngrp - 1)].append(fn)

        def step(g):
            ss = []
            sc = members(g + 1) if do_att and g + 1 < ngrp else []
            for c in _ORDER:
                if c == "S":
                    ss = [scores(p, sl) for p, sl in sc]
                elif c == "V" and do_att and g >= 0:
                    for p, sl in members(g):
                        pv(p, sl)
                elif c == "P" and do_att and g + 2 < ngrp:
                    for p, sl in members(g + 2):
                        proj(p, sl)
                elif c == "R":
                    for s_, (p, sl) in zip(ss, sc):
                        probs(s_, sl)
                elif c == "X":
                    for fn in side[g]:
                        fn()

        if do_att:
            for p, sl in members(0):
                proj(p, sl)
        for g in range(-1, ngrp):
            step(g)
        if do_att:
            for r in range(_WS):
                out_unit(r, ntile - 1)

    last = nstrips + 1
    parity = jax.lax.rem(t, 2)
    steady = jnp.logical_and(t >= 2, t < last)

    @pl.when(t == 0)
    def _first():
        main(0, 1, do_att=False, do_conv=False)

    @pl.when(t == 1)
    def _second():
        main(1, 0, do_att=False)

    @pl.when(jnp.logical_and(steady, parity == 0))
    def _even():
        main(0, 1)

    @pl.when(jnp.logical_and(steady, parity == 1))
    def _odd():
        main(1, 0)

    @pl.when(t == last)
    def _last():
        main(last % 2, 1 - last % 2, do_conv=False, do_stage=False)


@jax.jit
def pallas_standalone__window_attn_davit__vision_kernel(x, dw_pe, w_qkv, w_o):
    B, H, W, C = x.shape
    assert B == 1 and H % _WS == 0 and W % _WS == 0 and W + _WS + 1 <= 520 and C == 192
    nstrips = H // _WS
    WP = 512
    u32 = jnp.uint32
    xt = jnp.transpose(x, (0, 1, 3, 2)).reshape(H, C, W)
    dw = jnp.pad(dw_pe.reshape(9, C), ((0, 7), (0, 256 - C)))
    kern = functools.partial(_kernel, H=H, W=W, C=C, nstrips=nstrips)

    def strip(t):
        return jnp.minimum(t, nstrips - 1)

    out = pl.pallas_call(
        kern,
        grid=(nstrips + 2,),
        in_specs=[
            pl.BlockSpec((_WS, C, WP), lambda t: (strip(t), 0, 0)),
            pl.BlockSpec((1, C, WP), lambda t: (jnp.maximum(strip(t) * _WS - 1, 0), 0, 0)),
            pl.BlockSpec((1, C, WP), lambda t: (jnp.minimum(strip(t) * _WS + _WS, H - 1), 0, 0)),
            pl.BlockSpec((16, 256), lambda t: (0, 0)),
            pl.BlockSpec((C, 3 * C), lambda t: (0, 0)),
            pl.BlockSpec((C, C), lambda t: (0, 0)),
        ],
        out_specs=pl.BlockSpec((_WS, C, WP), lambda t: (jnp.maximum(t - 2, 0), 0, 0)),
        out_shape=jax.ShapeDtypeStruct((H, C, W), x.dtype),
        scratch_shapes=[
            pltpu.VMEM((9, C, 128), _F32),
            pltpu.VMEM((96, 256), u32),
            pltpu.VMEM((96, 256), u32),
            pltpu.VMEM((128, 256), u32),
            pltpu.VMEM((C // 2, 128), u32),
            pltpu.VMEM((C // 2, 128), u32),
            pltpu.VMEM((_WS + 2, C, WP), _F32),
            pltpu.VMEM((2, _WS, WP // 128, C, 128), _F32),
            pltpu.VMEM((2, 2, _WS, WP + 8, 128), _F32),
            pltpu.VMEM((2, 2, _WS, WP + 8, 128), _F32),
            pltpu.VMEM((_WS, WP + 8, 128), _F32),
            pltpu.VMEM((_WS, WP + 8, 128), _F32),
        ],
        compiler_params=pltpu.CompilerParams(
            dimension_semantics=("arbitrary",),
            vmem_limit_bytes=64 * 1024 * 1024,
        ),
    )(xt, xt, xt, dw, w_qkv, w_o)
    return jnp.transpose(out.reshape(1, H, C, W), (0, 1, 3, 2))
```

```python
import functools

import jax
import jax.numpy as jnp
import jax.experimental.pallas as pl
import jax.experimental.pallas.tpu as pltpu
import numpy as np

_WS = 7
_NH = 4
_NN = (((1,), (0,)), ((), ()))
_NT = (((1,), (1,)), ((), ()))
_F32 = jnp.float32
_BF16 = jnp.bfloat16
_NEG = -1e30
_GROUP = 2
_CSPAN = 14
_NLAG = 1
_CH = 48
_ORDER = "SnVPcRos"
_NORM0 = 1


def _dot(a, b, dims):
    return jax.lax.dot_general(a, b, dims, preferred_element_type=_F32)


def _xpose(a):
    r, c = a.shape
    rp, cp = -(-r // 128) * 128, -(-c // 128) * 128
    if rp != r:
        a = jnp.concatenate([a, jnp.zeros((rp - r, c), a.dtype)], axis=0)
    if cp != c:
        a = jnp.concatenate([a, jnp.zeros((rp, cp - c), a.dtype)], axis=1)
    return a.T[:c, :r]


def _pk(a):
    return pltpu.bitcast(a.astype(_BF16), jnp.uint32)


def _upk(a):
    return pltpu.bitcast(a, _BF16)


def _kernel(x_ref, xu_ref, xd_ref, dw_ref, wqkv_ref, wo_ref, o_ref,
            wconv_s, lab_s, lba_s, rk_s, loe_s, loo_s,
            xs_s, x0_s, h_s, k_s, oe_s, oo_s, *, H, W, C, nstrips):
    t = pl.program_id(0)
    dh = C // _NH
    WP = 512
    nwin = W // _WS
    npair = (nwin + 1) // 2
    CH = _CH
    nunit = _WS * (C // CH)

    @pl.when(t == 0)
    def _prep():
        def padk(a):
            return jnp.concatenate([a, jnp.zeros((a.shape[0], 256 - C), _F32)], axis=1)
        wT = _xpose(wqkv_ref[...].astype(_F32))
        lab_s[...] = _pk(padk(jnp.concatenate(
            [wT[0:dh], wT[2 * dh:3 * dh], wT[2 * C:2 * C + 2 * dh]], axis=0)))
        lba_s[...] = _pk(padk(jnp.concatenate(
            [wT[dh:2 * dh], wT[3 * dh:4 * dh], wT[2 * C + 2 * dh:3 * C]], axis=0)))
        z = jnp.zeros((128 - 2 * dh, C), _F32)
        kscale = float(dh) ** -0.5 * float(np.log2(np.e))
        k01 = jnp.concatenate([wT[C:C + 2 * dh] * kscale, z], axis=0)
        k23 = jnp.concatenate([wT[C + 2 * dh:2 * C] * kscale, z], axis=0)
        rk_s[...] = _pk(jnp.concatenate([padk(k01).T, padk(k23).T], axis=1))
        wo = wo_ref[...].astype(_F32)
        woe = jnp.concatenate([wo[0:dh], wo[2 * dh:3 * dh], z], axis=0)
        woo = jnp.concatenate([wo[dh:2 * dh], wo[3 * dh:4 * dh], z], axis=0)
        loe_s[...] = _pk(_xpose(woe))
        loo_s[...] = _pk(_xpose(woo))
        dwT = _xpose(dw_ref[...].astype(_F32))
        for k in range(9):
            wk = jnp.broadcast_to(dwT[0:C, k:k + 1], (C, 128))
            wconv_s[k] = wk + 1.0 if k == 4 else wk
        h_s[:, :, :, pl.ds(WP, 8), :] = jnp.zeros((2, 2, _WS, 8, 128), _F32)
        k_s[:, :, :, pl.ds(WP, 8), :] = jnp.zeros((2, 2, _WS, 8, 128), _F32)

    def main(bufB, bufA, do_att=True, do_conv=True, do_stage=True):
        lane = jax.lax.broadcasted_iota(jnp.int32, (1, 128), 1)
        last_ok = lane < (W - (WP - 128))

        def stage_row(dst, ref, ok, src=0):
            v = ref[src].astype(_F32)
            okl = last_ok if ok is None else jnp.logical_and(last_ok, ok)
            lo = v[:, :WP - 128] if ok is None else jnp.where(ok, v[:, :WP - 128], 0.0)
            xs_s[dst, :, :WP - 128] = lo
            xs_s[dst, :, WP - 128:] = jnp.where(okl, v[:, WP - 128:], 0.0)

        def conv_unit(u):
            r = u // (C // CH)
            c0 = (u - r * (C // CH)) * CH
            y = [None, None, None]
            for a in range(3):
                xv = xs_s[r + a, c0:c0 + CH, :]
                for b in range(3):
                    w = wconv_s[3 * a + b, c0:c0 + CH, :]
                    term = xv * jnp.concatenate([w] * (WP // 128), axis=1)
                    y[b] = term if y[b] is None else y[b] + term
            x0 = y[1] + (pltpu.roll(y[0], 1, 1) + pltpu.roll(y[2], WP - 1, 1))
            for j in range(WP // 128):
                x0_s[bufA, r, j, c0:c0 + CH, :] = x0[:, 128 * j:128 * (j + 1)]

        def norm_unit(r, j):
            x0 = x0_s[bufA, r, j]
            mean = jnp.sum(x0, axis=0, keepdims=True) * (1.0 / C)
            ex2 = jnp.sum(x0 * x0, axis=0, keepdims=True) * (1.0 / C)
            rstd = jax.lax.rsqrt(jnp.maximum(ex2 - mean * mean, 0.0) + 1e-5)
            hn = (x0 - mean) * rstd
            hb = jnp.concatenate([hn, jnp.zeros((256 - C, 128), _F32)], axis=0).astype(_BF16).T
            hf = hb.astype(_F32)
            h_s[bufA, 0, r, 128 * j:128 * (j + 1), :] = hf[:, 0:128]
            h_s[bufA, 1, r, 128 * j:128 * (j + 1), :] = hf[:, 128:256]
            kk = _dot(hb, _upk(rk_s[...]), _NN)
            k_s[bufA, 0, r, 128 * j:128 * (j + 1), :] = kk[:, 0:128]
            k_s[bufA, 1, r, 128 * j:128 * (j + 1), :] = kk[:, 128:256]

        def out_unit(r, j):
            sl = slice(128 * j, 128 * (j + 1))
            oe = oe_s[r, sl, :].astype(_BF16)
            oo = oo_s[r, sl, :].astype(_BF16)
            for m in range(2):
                a0, b0 = 48 * m, 96 * m
                y = (_dot(_upk(loe_s[a0:a0 + 48, :]), oe, _NT) + _dot(_upk(loo_s[a0:a0 + 48, :]), oo, _NT))
                o_ref[r, b0:b0 + 96, sl] = (x0_s[bufB, r, j, b0:b0 + 96, :] + y).astype(o_ref.dtype)

        left = lane < 64
        qv, pr = {}, {}

        def selL(a):
            return jnp.where(left, a, 0.0)

        def selR(a):
            return jnp.where(left, 0.0, a)

        key_ok = (jax.lax.broadcasted_iota(jnp.int32, (56, 128), 0) % 8) < _WS
        z8 = jnp.zeros((8, 256), _F32)
        z32 = jnp.zeros((32, 128), _F32)
        z8l = jnp.zeros((8, 128), _F32)

        def softmax_t(s):
            s = jnp.where(key_ok, s, _NEG)
            m = jnp.max(s, axis=0, keepdims=True)
            p = jnp.exp2(s - m)
            l = jnp.sum(p, axis=0, keepdims=True)
            r0 = pl.reciprocal(l, approx=True)
            r1 = r0 * (2.0 - l * r0)
            return p, r1 * (2.0 - l * r1)

        def gather(ref, t0):
            return [jnp.concatenate([ref[bufB, k, r, pl.ds(t0, 8), :] for r in range(_WS)], axis=0)
                    for k in range(2)]

        def proj(p, slot):
            ta_ = p * (2 * _WS)
            hA = jnp.concatenate(gather(h_s, ta_), axis=1)
            hB = jnp.concatenate(gather(h_s, ta_ + _WS), axis=1)
            hAB = jnp.concatenate([hA, z8, hB, z8], axis=0).astype(_BF16)
            hBA = jnp.concatenate([hB, z8, hA, z8], axis=0).astype(_BF16)
            r1 = _dot(_upk(lab_s[...]), hAB, _NT)
            r2 = _dot(_upk(lba_s[...]), hBA, _NT)
            qs = []
            for t2 in range(2):
                e = r1[dh * t2:dh * (t2 + 1)]
                o = r2[dh * t2:dh * (t2 + 1)]
                qs.append(jnp.concatenate([selL(e), selR(o)], axis=0).astype(_BF16))
                qs.append(jnp.concatenate([selR(e), selL(o)], axis=0).astype(_BF16))
            vs = [a[k * dh:(k + 1) * dh].astype(_BF16) for a in (r1, r2) for k in (2, 3)]
            qv[p] = (qs, vs)

        def scores(p, slot):
            ta_ = p * (2 * _WS)
            kA = gather(k_s, ta_)
            kB = gather(k_s, ta_ + _WS)
            out = []
            for t2 in range(2):
                sA = _dot(kA[t2][:, 0:96], qv[p][0][2 * t2], _NN)
                sB = _dot(kB[t2][:, 0:96], qv[p][0][2 * t2 + 1], _NN)
                out.append((sA, sB))
            return out

        def probs(ss, slot):
            out = []
            for t2 in range(2):
                pA, rA = softmax_t(ss[t2][0])
                pB, rB = softmax_t(ss[t2][1])
                pe, po = [selL(pA), z8l, selR(pB), z8l], [selR(pA), z8l, selL(pB), z8l]
                if t2 == 1:
                    pe, po = pe[2:] + pe[:2], po[2:] + po[:2]
                out.append((jnp.concatenate(pe, axis=0).astype(_BF16),
                            jnp.concatenate(po, axis=0).astype(_BF16),
                            jnp.where(left, rA, rB), jnp.where(left, rB, rA)))
            pr[slot] = out

        def pv(p, slot):
            ta_ = p * (2 * _WS)
            tb_ = ta_ + _WS
            oe, oo = [], []
            for t2 in range(2):
                pe, po, re_, ro_ = pr[p][t2]
                oe.append(_dot(qv[p][1][2 * t2], pe, _NN) * re_)
                oo.append(_dot(qv[p][1][2 * t2 + 1], po, _NN) * ro_)
            oeT = jnp.concatenate(oe + [z32], axis=0).astype(_BF16).T.astype(_F32)
            ooT = jnp.concatenate(oo + [z32], axis=0).astype(_BF16).T.astype(_F32)
            for r in range(_WS):
                oe_s[r, pl.ds(ta_, 8), :] = oeT[8 * r:8 * r + 8]
                oo_s[r, pl.ds(ta_, 8), :] = ooT[64 + 8 * r:64 + 8 * r + 8]
            for r in range(_WS):
                oe_s[r, pl.ds(tb_, 8), :] = oeT[64 + 8 * r:64 + 8 * r + 8]
                oo_s[r, pl.ds(tb_, 8), :] = ooT[8 * r:8 * r + 8]

        G = _GROUP
        ngrp = -(-npair // G)
        nslot = 3 * G
        ntile = WP // 128

        def members(g):
            return [(p, p) for p in range(g * G, min((g + 1) * G, npair))]

        side = {(k, g): [] for k in "cnos" for g in range(-1, ngrp)}
        conv_at = [-1 + (u * _CSPAN) // nunit for u in range(nunit)]
        conv_done = conv_at[-1] if do_conv else -2
        for u in range(nunit if do_conv else 0):
            side["c", conv_at[u]].append(functools.partial(conv_unit, u))
        nnorm = _WS * ntile
        for n in range(nnorm if do_conv else 0):
            r = n // ntile
            ready = conv_at[(C // CH) * (r + 1) - 1]
            g = max(ready + _NLAG, _NORM0 + (n * (ngrp - _NORM0)) // nnorm)
            side["n", min(g, ngrp - 1)].append(functools.partial(norm_unit, r, n % ntile))
        for j in range(ntile if do_att else 0):
            ready = min((128 * (j + 1) - 1) // (2 * _WS), npair - 1) // G
            nxt = min((128 * (j + 2) - 1) // (2 * _WS), npair - 1) // G if j + 1 < ntile else ready
            for r in range(_WS):
                g = ready + 1 + (r * (nxt - ready)) // _WS
                if g <= ngrp - 1:
                    side["o", g].append(functools.partial(out_unit, r, j))
        stages = [functools.partial(stage_row, 0, xu_ref, t > 0),
                  functools.partial(stage_row, _WS + 1, xd_ref, t < nstrips - 1)]
        stages += [functools.partial(stage_row, r + 1, x_ref, None, r) for r in range(_WS)]
        for n, fn in enumerate(stages if do_stage else []):
            g = conv_done + 1 + (n * (ngrp - 1 - conv_done)) // len(stages)
            side["s", min(g, ngrp - 1)].append(fn)

        def step(g):
            ss = []
            sc = members(g + 1) if do_att and g + 1 < ngrp else []
            for c in _ORDER:
                if c == "S":
                    ss = [scores(p, sl) for p, sl in sc]
                elif c == "V" and do_att and g >= 0:
                    for p, sl in members(g):
                        pv(p, sl)
                elif c == "P" and do_att and g + 2 < ngrp:
                    for p, sl in members(g + 2):
                        proj(p, sl)
                elif c == "R":
                    for s_, (p, sl) in zip(ss, sc):
                        probs(s_, sl)
                elif c in "cnos":
                    for fn in side[c, g]:
                        fn()

        if do_att:
            for p, sl in members(0):
                proj(p, sl)
        for g in range(-1, ngrp):
            step(g)
        if do_att:
            for r in range(_WS):
                out_unit(r, ntile - 1)

    last = nstrips + 1
    parity = jax.lax.rem(t, 2)
    steady = jnp.logical_and(t >= 2, t < last)

    @pl.when(t == 0)
    def _first():
        main(0, 1, do_att=False, do_conv=False)

    @pl.when(t == 1)
    def _second():
        main(1, 0, do_att=False)

    @pl.when(jnp.logical_and(steady, parity == 0))
    def _even():
        main(0, 1)

    @pl.when(jnp.logical_and(steady, parity == 1))
    def _odd():
        main(1, 0)

    @pl.when(t == last)
    def _last():
        main(last % 2, 1 - last % 2, do_conv=False, do_stage=False)


@jax.jit
def pallas_standalone__window_attn_davit__vision_kernel(x, dw_pe, w_qkv, w_o):
    B, H, W, C = x.shape
    assert B == 1 and H % _WS == 0 and W % _WS == 0 and W + _WS + 1 <= 520 and C == 192
    nstrips = H // _WS
    WP = 512
    u32 = jnp.uint32
    xt = jnp.transpose(x, (0, 1, 3, 2)).reshape(H, C, W)
    dw = jnp.pad(dw_pe.reshape(9, C), ((0, 7), (0, 256 - C)))
    kern = functools.partial(_kernel, H=H, W=W, C=C, nstrips=nstrips)

    def strip(t):
        return jnp.minimum(t, nstrips - 1)

    out = pl.pallas_call(
        kern,
        grid=(nstrips + 2,),
        in_specs=[
            pl.BlockSpec((_WS, C, WP), lambda t: (strip(t), 0, 0)),
            pl.BlockSpec((1, C, WP), lambda t: (jnp.maximum(strip(t) * _WS - 1, 0), 0, 0)),
            pl.BlockSpec((1, C, WP), lambda t: (jnp.minimum(strip(t) * _WS + _WS, H - 1), 0, 0)),
            pl.BlockSpec((16, 256), lambda t: (0, 0)),
            pl.BlockSpec((C, 3 * C), lambda t: (0, 0)),
            pl.BlockSpec((C, C), lambda t: (0, 0)),
        ],
        out_specs=pl.BlockSpec((_WS, C, WP), lambda t: (jnp.maximum(t - 2, 0), 0, 0)),
        out_shape=jax.ShapeDtypeStruct((H, C, W), x.dtype),
        scratch_shapes=[
            pltpu.VMEM((9, C, 128), _F32),
            pltpu.VMEM((96, 256), u32),
            pltpu.VMEM((96, 256), u32),
            pltpu.VMEM((128, 256), u32),
            pltpu.VMEM((C // 2, 128), u32),
            pltpu.VMEM((C // 2, 128), u32),
            pltpu.VMEM((_WS + 2, C, WP), _F32),
            pltpu.VMEM((2, _WS, WP // 128, C, 128), _F32),
            pltpu.VMEM((2, 2, _WS, WP + 8, 128), _F32),
            pltpu.VMEM((2, 2, _WS, WP + 8, 128), _F32),
            pltpu.VMEM((_WS, WP + 8, 128), _F32),
            pltpu.VMEM((_WS, WP + 8, 128), _F32),
        ],
        compiler_params=pltpu.CompilerParams(
            dimension_semantics=("arbitrary",),
            vmem_limit_bytes=64 * 1024 * 1024,
        ),
    )(xt, xt, xt, dw, w_qkv, w_o)
    return jnp.transpose(out.reshape(1, H, C, W), (0, 1, 3, 2))
```

```python
import functools

import jax
import jax.numpy as jnp
import jax.experimental.pallas as pl
import jax.experimental.pallas.tpu as pltpu
import numpy as np

_WS = 7
_NH = 4
_NN = (((1,), (0,)), ((), ()))
_NT = (((1,), (1,)), ((), ()))
_F32 = jnp.float32
_BF16 = jnp.bfloat16
_NEG = -1e30
_GROUP = 2
_CSPAN = 14
_NLAG = 1
_S0 = -1
_SSPAN = 19
_CH = 48
_ORDER = "ScVPnRos"
_NORM0 = 1


def _dot(a, b, dims):
    return jax.lax.dot_general(a, b, dims, preferred_element_type=_F32)


def _xpose(a):
    r, c = a.shape
    rp, cp = -(-r // 128) * 128, -(-c // 128) * 128
    if rp != r:
        a = jnp.concatenate([a, jnp.zeros((rp - r, c), a.dtype)], axis=0)
    if cp != c:
        a = jnp.concatenate([a, jnp.zeros((rp, cp - c), a.dtype)], axis=1)
    return a.T[:c, :r]


def _pk(a):
    return pltpu.bitcast(a.astype(_BF16), jnp.uint32)


def _upk(a):
    return pltpu.bitcast(a, _BF16)


def _kernel(x_ref, xu_ref, xd_ref, dw_ref, wqkv_ref, wo_ref, o_ref,
            wconv_s, lab_s, lba_s, rk_s, loe_s, loo_s,
            xs_s, x0_s, h_s, k_s, oe_s, oo_s, *, H, W, C, nstrips):
    t = pl.program_id(0)
    dh = C // _NH
    WP = 512
    nwin = W // _WS
    npair = (nwin + 1) // 2
    CH = _CH
    nunit = _WS * (C // CH)

    @pl.when(t == 0)
    def _prep():
        def padk(a):
            return jnp.concatenate([a, jnp.zeros((a.shape[0], 256 - C), _F32)], axis=1)
        wT = _xpose(wqkv_ref[...].astype(_F32))
        lab_s[...] = _pk(padk(jnp.concatenate(
            [wT[0:dh], wT[2 * dh:3 * dh], wT[2 * C:2 * C + 2 * dh]], axis=0)))
        lba_s[...] = _pk(padk(jnp.concatenate(
            [wT[dh:2 * dh], wT[3 * dh:4 * dh], wT[2 * C + 2 * dh:3 * C]], axis=0)))
        z = jnp.zeros((128 - 2 * dh, C), _F32)
        kscale = float(dh) ** -0.5 * float(np.log2(np.e))
        k01 = jnp.concatenate([wT[C:C + 2 * dh] * kscale, z], axis=0)
        k23 = jnp.concatenate([wT[C + 2 * dh:2 * C] * kscale, z], axis=0)
        rk_s[...] = _pk(jnp.concatenate([padk(k01).T, padk(k23).T], axis=1))
        wo = wo_ref[...].astype(_F32)
        woe = jnp.concatenate([wo[0:dh], wo[2 * dh:3 * dh], z], axis=0)
        woo = jnp.concatenate([wo[dh:2 * dh], wo[3 * dh:4 * dh], z], axis=0)
        loe_s[...] = _pk(_xpose(woe))
        loo_s[...] = _pk(_xpose(woo))
        dwT = _xpose(dw_ref[...].astype(_F32))
        for k in range(9):
            wk = jnp.broadcast_to(dwT[0:C, k:k + 1], (C, 128))
            wconv_s[k] = wk + 1.0 if k == 4 else wk
        h_s[:, :, :, pl.ds(WP, 8), :] = jnp.zeros((2, 2, _WS, 8, 128), _F32)
        k_s[:, :, :, pl.ds(WP, 8), :] = jnp.zeros((2, 2, _WS, 8, 128), _F32)

    def main(bufB, bufA, do_att=True, do_conv=True, do_stage=True):
        lane = jax.lax.broadcasted_iota(jnp.int32, (1, 128), 1)
        last_ok = lane < (W - (WP - 128))

        def stage_row(dst, ref, ok, src=0):
            v = ref[src].astype(_F32)
            okl = last_ok if ok is None else jnp.logical_and(last_ok, ok)
            lo = v[:, :WP - 128] if ok is None else jnp.where(ok, v[:, :WP - 128], 0.0)
            xs_s[bufB, dst, :, :WP - 128] = lo
            xs_s[bufB, dst, :, WP - 128:] = jnp.where(okl, v[:, WP - 128:], 0.0)

        def conv_unit(u):
            r = u // (C // CH)
            c0 = (u - r * (C // CH)) * CH
            y = [None, None, None]
            for a in range(3):
                xv = xs_s[bufA, r + a, c0:c0 + CH, :]
                for b in range(3):
                    w = wconv_s[3 * a + b, c0:c0 + CH, :]
                    term = xv * jnp.concatenate([w] * (WP // 128), axis=1)
                    y[b] = term if y[b] is None else y[b] + term
            x0 = y[1] + (pltpu.roll(y[0], 1, 1) + pltpu.roll(y[2], WP - 1, 1))
            for j in range(WP // 128):
                x0_s[bufA, r, j, c0:c0 + CH, :] = x0[:, 128 * j:128 * (j + 1)]

        def norm_unit(r, j):
            x0 = x0_s[bufA, r, j]
            mean = jnp.sum(x0, axis=0, keepdims=True) * (1.0 / C)
            ex2 = jnp.sum(x0 * x0, axis=0, keepdims=True) * (1.0 / C)
            rstd = jax.lax.rsqrt(jnp.maximum(ex2 - mean * mean, 0.0) + 1e-5)
            hn = (x0 - mean) * rstd
            hb = jnp.concatenate([hn, jnp.zeros((256 - C, 128), _F32)], axis=0).astype(_BF16).T
            hf = hb.astype(_F32)
            h_s[bufA, 0, r, 128 * j:128 * (j + 1), :] = hf[:, 0:128]
            h_s[bufA, 1, r, 128 * j:128 * (j + 1), :] = hf[:, 128:256]
            kk = _dot(hb, _upk(rk_s[...]), _NN)
            k_s[bufA, 0, r, 128 * j:128 * (j + 1), :] = kk[:, 0:128]
            k_s[bufA, 1, r, 128 * j:128 * (j + 1), :] = kk[:, 128:256]

        def out_unit(r, j):
            sl = slice(128 * j, 128 * (j + 1))
            oe = oe_s[r, sl, :].astype(_BF16)
            oo = oo_s[r, sl, :].astype(_BF16)
            for m in range(2):
                a0, b0 = 48 * m, 96 * m
                y = (_dot(_upk(loe_s[a0:a0 + 48, :]), oe, _NT) + _dot(_upk(loo_s[a0:a0 + 48, :]), oo, _NT))
                o_ref[r, b0:b0 + 96, sl] = (x0_s[bufB, r, j, b0:b0 + 96, :] + y).astype(o_ref.dtype)

        left = lane < 64
        qv, pr = {}, {}

        def selL(a):
            return jnp.where(left, a, 0.0)

        def selR(a):
            return jnp.where(left, 0.0, a)

        key_ok = (jax.lax.broadcasted_iota(jnp.int32, (56, 128), 0) % 8) < _WS
        z8 = jnp.zeros((8, 256), _F32)
        z32 = jnp.zeros((32, 128), _F32)
        z8l = jnp.zeros((8, 128), _F32)

        def softmax_t(s):
            s = jnp.where(key_ok, s, _NEG)
            m = jnp.max(s, axis=0, keepdims=True)
            p = jnp.exp2(s - m)
            l = jnp.sum(p, axis=0, keepdims=True)
            r0 = pl.reciprocal(l, approx=True)
            r1 = r0 * (2.0 - l * r0)
            return p, r1 * (2.0 - l * r1)

        def gather(ref, t0):
            return [jnp.concatenate([ref[bufB, k, r, pl.ds(t0, 8), :] for r in range(_WS)], axis=0)
                    for k in range(2)]

        def proj(p, slot):
            ta_ = p * (2 * _WS)
            hA = jnp.concatenate(gather(h_s, ta_), axis=1)
            hB = jnp.concatenate(gather(h_s, ta_ + _WS), axis=1)
            hAB = jnp.concatenate([hA, z8, hB, z8], axis=0).astype(_BF16)
            hBA = jnp.concatenate([hB, z8, hA, z8], axis=0).astype(_BF16)
            r1 = _dot(_upk(lab_s[...]), hAB, _NT)
            r2 = _dot(_upk(lba_s[...]), hBA, _NT)
            qs = []
            for t2 in range(2):
                e = r1[dh * t2:dh * (t2 + 1)]
                o = r2[dh * t2:dh * (t2 + 1)]
                qs.append(jnp.concatenate([selL(e), selR(o)], axis=0).astype(_BF16))
                qs.append(jnp.concatenate([selR(e), selL(o)], axis=0).astype(_BF16))
            vs = [a[k * dh:(k + 1) * dh].astype(_BF16) for a in (r1, r2) for k in (2, 3)]
            qv[p] = (qs, vs)

        def scores(p, slot):
            ta_ = p * (2 * _WS)
            kA = gather(k_s, ta_)
            kB = gather(k_s, ta_ + _WS)
            out = []
            for t2 in range(2):
                sA = _dot(kA[t2][:, 0:96], qv[p][0][2 * t2], _NN)
                sB = _dot(kB[t2][:, 0:96], qv[p][0][2 * t2 + 1], _NN)
                out.append((sA, sB))
            return out

        def probs(ss, slot):
            out = []
            for t2 in range(2):
                pA, rA = softmax_t(ss[t2][0])
                pB, rB = softmax_t(ss[t2][1])
                pe, po = [selL(pA), z8l, selR(pB), z8l], [selR(pA), z8l, selL(pB), z8l]
                if t2 == 1:
                    pe, po = pe[2:] + pe[:2], po[2:] + po[:2]
                out.append((jnp.concatenate(pe, axis=0).astype(_BF16),
                            jnp.concatenate(po, axis=0).astype(_BF16),
                            jnp.where(left, rA, rB), jnp.where(left, rB, rA)))
            pr[slot] = out

        def pv(p, slot):
            ta_ = p * (2 * _WS)
            tb_ = ta_ + _WS
            oe, oo = [], []
            for t2 in range(2):
                pe, po, re_, ro_ = pr[p][t2]
                oe.append(_dot(qv[p][1][2 * t2], pe, _NN) * re_)
                oo.append(_dot(qv[p][1][2 * t2 + 1], po, _NN) * ro_)
            oeT = jnp.concatenate(oe + [z32], axis=0).astype(_BF16).T.astype(_F32)
            ooT = jnp.concatenate(oo + [z32], axis=0).astype(_BF16).T.astype(_F32)
            for r in range(_WS):
                oe_s[r, pl.ds(ta_, 8), :] = oeT[8 * r:8 * r + 8]
                oo_s[r, pl.ds(ta_, 8), :] = ooT[64 + 8 * r:64 + 8 * r + 8]
            for r in range(_WS):
                oe_s[r, pl.ds(tb_, 8), :] = oeT[64 + 8 * r:64 + 8 * r + 8]
                oo_s[r, pl.ds(tb_, 8), :] = ooT[8 * r:8 * r + 8]

        G = _GROUP
        ngrp = -(-npair // G)
        nslot = 3 * G
        ntile = WP // 128

        def members(g):
            return [(p, p) for p in range(g * G, min((g + 1) * G, npair))]

        side = {(k, g): [] for k in "cnos" for g in range(-1, ngrp)}
        conv_at = [-1 + (u * _CSPAN) // nunit for u in range(nunit)]
        conv_done = conv_at[-1] if do_conv else -2
        for u in range(nunit if do_conv else 0):
            side["c", conv_at[u]].append(functools.partial(conv_unit, u))
        nnorm = _WS * ntile
        for n in range(nnorm if do_conv else 0):
            r = n // ntile
            ready = conv_at[(C // CH) * (r + 1) - 1]
            g = max(ready + _NLAG, _NORM0 + (n * (ngrp - _NORM0)) // nnorm)
            side["n", min(g, ngrp - 1)].append(functools.partial(norm_unit, r, n % ntile))
        for j in range(ntile if do_att else 0):
            ready = min((128 * (j + 1) - 1) // (2 * _WS), npair - 1) // G
            nxt = min((128 * (j + 2) - 1) // (2 * _WS), npair - 1) // G if j + 1 < ntile else ready
            for r in range(_WS):
                g = ready + 1 + (r * (nxt - ready)) // _WS
                if g <= ngrp - 1:
                    side["o", g].append(functools.partial(out_unit, r, j))
        stages = [functools.partial(stage_row, 0, xu_ref, t > 0),
                  functools.partial(stage_row, _WS + 1, xd_ref, t < nstrips - 1)]
        stages += [functools.partial(stage_row, r + 1, x_ref, None, r) for r in range(_WS)]
        for n, fn in enumerate(stages if do_stage else []):
            g = _S0 + (n * _SSPAN) // len(stages)
            g = g if do_att else -1
            side["s", min(g, ngrp - 1)].append(fn)

        def step(g):
            ss = []
            sc = members(g + 1) if do_att and g + 1 < ngrp else []
            for c in _ORDER:
                if c == "S":
                    ss = [scores(p, sl) for p, sl in sc]
                elif c == "V" and do_att and g >= 0:
                    for p, sl in members(g):
                        pv(p, sl)
                elif c == "P" and do_att and g + 2 < ngrp:
                    for p, sl in members(g + 2):
                        proj(p, sl)
                elif c == "R":
                    for s_, (p, sl) in zip(ss, sc):
                        probs(s_, sl)
                elif c in "cnos":
                    for fn in side[c, g]:
                        fn()

        if do_att:
            for p, sl in members(0):
                proj(p, sl)
        for g in range(-1, ngrp):
            step(g)
        if do_att:
            for r in range(_WS):
                out_unit(r, ntile - 1)

    last = nstrips + 1
    parity = jax.lax.rem(t, 2)
    steady = jnp.logical_and(t >= 2, t < last)

    @pl.when(t == 0)
    def _first():
        main(0, 1, do_att=False, do_conv=False)

    @pl.when(t == 1)
    def _second():
        main(1, 0, do_att=False)

    @pl.when(jnp.logical_and(steady, parity == 0))
    def _even():
        main(0, 1)

    @pl.when(jnp.logical_and(steady, parity == 1))
    def _odd():
        main(1, 0)

    @pl.when(t == last)
    def _last():
        main(last % 2, 1 - last % 2, do_conv=False, do_stage=False)


@jax.jit
def pallas_standalone__window_attn_davit__vision_kernel(x, dw_pe, w_qkv, w_o):
    B, H, W, C = x.shape
    assert B == 1 and H % _WS == 0 and W % _WS == 0 and W + _WS + 1 <= 520 and C == 192
    nstrips = H // _WS
    WP = 512
    u32 = jnp.uint32
    xt = jnp.transpose(x, (0, 1, 3, 2)).reshape(H, C, W)
    dw = jnp.pad(dw_pe.reshape(9, C), ((0, 7), (0, 256 - C)))
    kern = functools.partial(_kernel, H=H, W=W, C=C, nstrips=nstrips)

    def strip(t):
        return jnp.minimum(t, nstrips - 1)

    out = pl.pallas_call(
        kern,
        grid=(nstrips + 2,),
        in_specs=[
            pl.BlockSpec((_WS, C, WP), lambda t: (strip(t), 0, 0)),
            pl.BlockSpec((1, C, WP), lambda t: (jnp.maximum(strip(t) * _WS - 1, 0), 0, 0)),
            pl.BlockSpec((1, C, WP), lambda t: (jnp.minimum(strip(t) * _WS + _WS, H - 1), 0, 0)),
            pl.BlockSpec((16, 256), lambda t: (0, 0)),
            pl.BlockSpec((C, 3 * C), lambda t: (0, 0)),
            pl.BlockSpec((C, C), lambda t: (0, 0)),
        ],
        out_specs=pl.BlockSpec((_WS, C, WP), lambda t: (jnp.maximum(t - 2, 0), 0, 0)),
        out_shape=jax.ShapeDtypeStruct((H, C, W), x.dtype),
        scratch_shapes=[
            pltpu.VMEM((9, C, 128), _F32),
            pltpu.VMEM((96, 256), u32),
            pltpu.VMEM((96, 256), u32),
            pltpu.VMEM((128, 256), u32),
            pltpu.VMEM((C // 2, 128), u32),
            pltpu.VMEM((C // 2, 128), u32),
            pltpu.VMEM((2, _WS + 2, C, WP), _F32),
            pltpu.VMEM((2, _WS, WP // 128, C, 128), _F32),
            pltpu.VMEM((2, 2, _WS, WP + 8, 128), _F32),
            pltpu.VMEM((2, 2, _WS, WP + 8, 128), _F32),
            pltpu.VMEM((_WS, WP + 8, 128), _F32),
            pltpu.VMEM((_WS, WP + 8, 128), _F32),
        ],
        compiler_params=pltpu.CompilerParams(
            dimension_semantics=("arbitrary",),
            vmem_limit_bytes=64 * 1024 * 1024,
        ),
    )(xt, xt, xt, dw, w_qkv, w_o)
    return jnp.transpose(out.reshape(1, H, C, W), (0, 1, 3, 2))
```

```python
import functools

import jax
import jax.numpy as jnp
import jax.experimental.pallas as pl
import jax.experimental.pallas.tpu as pltpu
import numpy as np

_WS = 7
_NH = 4
_NN = (((1,), (0,)), ((), ()))
_NT = (((1,), (1,)), ((), ()))
_F32 = jnp.float32
_BF16 = jnp.bfloat16
_NEG = -1e30
_GROUP = 2
_CSPAN = 14
_NLAG = 1
_NSPAN = 26
_ODIV = 7
_S0 = -1
_SSPAN = 19
_CH = 48
_ORDER = "ScVPnRos"
_NORM0 = 1


def _dot(a, b, dims):
    return jax.lax.dot_general(a, b, dims, preferred_element_type=_F32)


def _xpose(a):
    r, c = a.shape
    rp, cp = -(-r // 128) * 128, -(-c // 128) * 128
    if rp != r:
        a = jnp.concatenate([a, jnp.zeros((rp - r, c), a.dtype)], axis=0)
    if cp != c:
        a = jnp.concatenate([a, jnp.zeros((rp, cp - c), a.dtype)], axis=1)
    return a.T[:c, :r]


def _pk(a):
    return pltpu.bitcast(a.astype(_BF16), jnp.uint32)


def _upk(a):
    return pltpu.bitcast(a, _BF16)


def _kernel(x_ref, xu_ref, xd_ref, dw_ref, wqkv_ref, wo_ref, o_ref,
            wconv_s, lab_s, lba_s, rk_s, loe_s, loo_s,
            xs_s, x0_s, h_s, k_s, oe_s, oo_s, *, H, W, C, nstrips):
    t = pl.program_id(0)
    dh = C // _NH
    WP = 512
    nwin = W // _WS
    npair = (nwin + 1) // 2
    CH = _CH
    nunit = _WS * (C // CH)

    @pl.when(t == 0)
    def _prep():
        def padk(a):
            return jnp.concatenate([a, jnp.zeros((a.shape[0], 256 - C), _F32)], axis=1)
        wT = _xpose(wqkv_ref[...].astype(_F32))
        lab_s[...] = _pk(padk(jnp.concatenate(
            [wT[0:dh], wT[2 * dh:3 * dh], wT[2 * C:2 * C + 2 * dh]], axis=0)))
        lba_s[...] = _pk(padk(jnp.concatenate(
            [wT[dh:2 * dh], wT[3 * dh:4 * dh], wT[2 * C + 2 * dh:3 * C]], axis=0)))
        z = jnp.zeros((128 - 2 * dh, C), _F32)
        kscale = float(dh) ** -0.5 * float(np.log2(np.e))
        k01 = jnp.concatenate([wT[C:C + 2 * dh] * kscale, z], axis=0)
        k23 = jnp.concatenate([wT[C + 2 * dh:2 * C] * kscale, z], axis=0)
        rk_s[...] = _pk(jnp.concatenate([padk(k01).T, padk(k23).T], axis=1))
        wo = wo_ref[...].astype(_F32)
        woe = jnp.concatenate([wo[0:dh], wo[2 * dh:3 * dh], z], axis=0)
        woo = jnp.concatenate([wo[dh:2 * dh], wo[3 * dh:4 * dh], z], axis=0)
        loe_s[...] = _pk(_xpose(woe))
        loo_s[...] = _pk(_xpose(woo))
        dwT = _xpose(dw_ref[...].astype(_F32))
        for k in range(9):
            wk = jnp.broadcast_to(dwT[0:C, k:k + 1], (C, 128))
            wconv_s[k] = wk + 1.0 if k == 4 else wk
        h_s[:, :, :, pl.ds(WP, 8), :] = jnp.zeros((2, 2, _WS, 8, 128), _F32)
        k_s[:, :, :, pl.ds(WP, 8), :] = jnp.zeros((2, 2, _WS, 8, 128), _F32)

    def main(bufB, bufA, do_att=True, do_conv=True, do_stage=True):
        lane = jax.lax.broadcasted_iota(jnp.int32, (1, 128), 1)
        last_ok = lane < (W - (WP - 128))

        def stage_row(dst, ref, ok, src=0):
            v = ref[src].astype(_F32)
            okl = last_ok if ok is None else jnp.logical_and(last_ok, ok)
            lo = v[:, :WP - 128] if ok is None else jnp.where(ok, v[:, :WP - 128], 0.0)
            xs_s[bufB, dst, :, :WP - 128] = lo
            xs_s[bufB, dst, :, WP - 128:] = jnp.where(okl, v[:, WP - 128:], 0.0)

        def conv_unit(u):
            r = u // (C // CH)
            c0 = (u - r * (C // CH)) * CH
            y = [None, None, None]
            for a in range(3):
                xv = xs_s[bufA, r + a, c0:c0 + CH, :]
                for b in range(3):
                    w = wconv_s[3 * a + b, c0:c0 + CH, :]
                    term = xv * jnp.concatenate([w] * (WP // 128), axis=1)
                    y[b] = term if y[b] is None else y[b] + term
            x0 = y[1] + (pltpu.roll(y[0], 1, 1) + pltpu.roll(y[2], WP - 1, 1))
            for j in range(WP // 128):
                x0_s[bufA, r, j, c0:c0 + CH, :] = x0[:, 128 * j:128 * (j + 1)]

        def norm_unit(r, j):
            x0 = x0_s[bufA, r, j]
            mean = jnp.sum(x0, axis=0, keepdims=True) * (1.0 / C)
            ex2 = jnp.sum(x0 * x0, axis=0, keepdims=True) * (1.0 / C)
            rstd = jax.lax.rsqrt(jnp.maximum(ex2 - mean * mean, 0.0) + 1e-5)
            hn = (x0 - mean) * rstd
            hb = jnp.concatenate([hn, jnp.zeros((256 - C, 128), _F32)], axis=0).astype(_BF16).T
            hf = hb.astype(_F32)
            h_s[bufA, 0, r, 128 * j:128 * (j + 1), :] = hf[:, 0:128]
            h_s[bufA, 1, r, 128 * j:128 * (j + 1), :] = hf[:, 128:256]
            kk = _dot(hb, _upk(rk_s[...]), _NN)
            k_s[bufA, 0, r, 128 * j:128 * (j + 1), :] = kk[:, 0:128]
            k_s[bufA, 1, r, 128 * j:128 * (j + 1), :] = kk[:, 128:256]

        def out_unit(r, j):
            sl = slice(128 * j, 128 * (j + 1))
            oe = oe_s[r, sl, :].astype(_BF16)
            oo = oo_s[r, sl, :].astype(_BF16)
            for m in range(2):
                a0, b0 = 48 * m, 96 * m
                y = (_dot(_upk(loe_s[a0:a0 + 48, :]), oe, _NT) + _dot(_upk(loo_s[a0:a0 + 48, :]), oo, _NT))
                o_ref[r, b0:b0 + 96, sl] = (x0_s[bufB, r, j, b0:b0 + 96, :] + y).astype(o_ref.dtype)

        left = lane < 64
        qv, pr = {}, {}

        def selL(a):
            return jnp.where(left, a, 0.0)

        def selR(a):
            return jnp.where(left, 0.0, a)

        key_ok = (jax.lax.broadcasted_iota(jnp.int32, (56, 128), 0) % 8) < _WS
        z8 = jnp.zeros((8, 256), _F32)
        z32 = jnp.zeros((32, 128), _F32)
        z8l = jnp.zeros((8, 128), _F32)

        def softmax_t(s):
            s = jnp.where(key_ok, s, _NEG)
            m = jnp.max(s, axis=0, keepdims=True)
            p = jnp.exp2(s - m)
            l = jnp.sum(p, axis=0, keepdims=True)
            r0 = pl.reciprocal(l, approx=True)
            r1 = r0 * (2.0 - l * r0)
            return p, r1 * (2.0 - l * r1)

        def gather(ref, t0):
            return [jnp.concatenate([ref[bufB, k, r, pl.ds(t0, 8), :] for r in range(_WS)], axis=0)
                    for k in range(2)]

        def proj(p, slot):
            ta_ = p * (2 * _WS)
            hA = jnp.concatenate(gather(h_s, ta_), axis=1)
            hB = jnp.concatenate(gather(h_s, ta_ + _WS), axis=1)
            hAB = jnp.concatenate([hA, z8, hB, z8], axis=0).astype(_BF16)
            hBA = jnp.concatenate([hB, z8, hA, z8], axis=0).astype(_BF16)
            r1 = _dot(_upk(lab_s[...]), hAB, _NT)
            r2 = _dot(_upk(lba_s[...]), hBA, _NT)
            qs = []
            for t2 in range(2):
                e = r1[dh * t2:dh * (t2 + 1)]
                o = r2[dh * t2:dh * (t2 + 1)]
                qs.append(jnp.concatenate([selL(e), selR(o)], axis=0).astype(_BF16))
                qs.append(jnp.concatenate([selR(e), selL(o)], axis=0).astype(_BF16))
            vs = [a[k * dh:(k + 1) * dh].astype(_BF16) for a in (r1, r2) for k in (2, 3)]
            qv[p] = (qs, vs)

        def scores(p, slot):
            ta_ = p * (2 * _WS)
            kA = gather(k_s, ta_)
            kB = gather(k_s, ta_ + _WS)
            out = []
            for t2 in range(2):
                sA = _dot(kA[t2][:, 0:96], qv[p][0][2 * t2], _NN)
                sB = _dot(kB[t2][:, 0:96], qv[p][0][2 * t2 + 1], _NN)
                out.append((sA, sB))
            return out

        def probs(ss, slot):
            out = []
            for t2 in range(2):
                pA, rA = softmax_t(ss[t2][0])
                pB, rB = softmax_t(ss[t2][1])
                pe, po = [selL(pA), z8l, selR(pB), z8l], [selR(pA), z8l, selL(pB), z8l]
                if t2 == 1:
                    pe, po = pe[2:] + pe[:2], po[2:] + po[:2]
                out.append((jnp.concatenate(pe, axis=0).astype(_BF16),
                            jnp.concatenate(po, axis=0).astype(_BF16),
                            jnp.where(left, rA, rB), jnp.where(left, rB, rA)))
            pr[slot] = out

        def pv(p, slot):
            ta_ = p * (2 * _WS)
            tb_ = ta_ + _WS
            oe, oo = [], []
            for t2 in range(2):
                pe, po, re_, ro_ = pr[p][t2]
                oe.append(_dot(qv[p][1][2 * t2], pe, _NN) * re_)
                oo.append(_dot(qv[p][1][2 * t2 + 1], po, _NN) * ro_)
            oeT = jnp.concatenate(oe + [z32], axis=0).astype(_BF16).T.astype(_F32)
            ooT = jnp.concatenate(oo + [z32], axis=0).astype(_BF16).T.astype(_F32)
            for r in range(_WS):
                oe_s[r, pl.ds(ta_, 8), :] = oeT[8 * r:8 * r + 8]
                oo_s[r, pl.ds(ta_, 8), :] = ooT[64 + 8 * r:64 + 8 * r + 8]
            for r in range(_WS):
                oe_s[r, pl.ds(tb_, 8), :] = oeT[64 + 8 * r:64 + 8 * r + 8]
                oo_s[r, pl.ds(tb_, 8), :] = ooT[8 * r:8 * r + 8]

        G = _GROUP
        ngrp = -(-npair // G)
        nslot = 3 * G
        ntile = WP // 128

        def members(g):
            return [(p, p) for p in range(g * G, min((g + 1) * G, npair))]

        side = {(k, g): [] for k in "cnos" for g in range(-1, ngrp)}
        conv_at = [-1 + (u * _CSPAN) // nunit for u in range(nunit)]
        conv_done = conv_at[-1] if do_conv else -2
        for u in range(nunit if do_conv else 0):
            side["c", conv_at[u]].append(functools.partial(conv_unit, u))
        nnorm = _WS * ntile
        for n in range(nnorm if do_conv else 0):
            r = n // ntile
            ready = conv_at[(C // CH) * (r + 1) - 1]
            g = max(ready + _NLAG, _NORM0 + (n * _NSPAN) // nnorm)
            side["n", min(g, ngrp - 1)].append(functools.partial(norm_unit, r, n % ntile))
        for j in range(ntile if do_att else 0):
            ready = min((128 * (j + 1) - 1) // (2 * _WS), npair - 1) // G
            nxt = min((128 * (j + 2) - 1) // (2 * _WS), npair - 1) // G if j + 1 < ntile else ready
            for r in range(_WS):
                g = ready + 1 + (r * (nxt - ready)) // _ODIV
                if g <= ngrp - 1:
                    side["o", g].append(functools.partial(out_unit, r, j))
        stages = [functools.partial(stage_row, 0, xu_ref, t > 0),
                  functools.partial(stage_row, _WS + 1, xd_ref, t < nstrips - 1)]
        stages += [functools.partial(stage_row, r + 1, x_ref, None, r) for r in range(_WS)]
        for n, fn in enumerate(stages if do_stage else []):
            g = _S0 + (n * _SSPAN) // len(stages)
            g = g if do_att else -1
            side["s", min(g, ngrp - 1)].append(fn)

        def step(g):
            ss = []
            sc = members(g + 1) if do_att and g + 1 < ngrp else []
            for c in _ORDER:
                if c == "S":
                    ss = [scores(p, sl) for p, sl in sc]
                elif c == "V" and do_att and g >= 0:
                    for p, sl in members(g):
                        pv(p, sl)
                elif c == "P" and do_att and g + 2 < ngrp:
                    for p, sl in members(g + 2):
                        proj(p, sl)
                elif c == "R":
                    for s_, (p, sl) in zip(ss, sc):
                        probs(s_, sl)
                elif c in "cnos":
                    for fn in side[c, g]:
                        fn()

        if do_att:
            for p, sl in members(0):
                proj(p, sl)
        for g in range(-1, ngrp):
            step(g)
        if do_att:
            for r in range(_WS):
                out_unit(r, ntile - 1)

    last = nstrips + 1
    parity = jax.lax.rem(t, 2)
    steady = jnp.logical_and(t >= 2, t < last)

    @pl.when(t == 0)
    def _first():
        main(0, 1, do_att=False, do_conv=False)

    @pl.when(t == 1)
    def _second():
        main(1, 0, do_att=False)

    @pl.when(jnp.logical_and(steady, parity == 0))
    def _even():
        main(0, 1)

    @pl.when(jnp.logical_and(steady, parity == 1))
    def _odd():
        main(1, 0)

    @pl.when(t == last)
    def _last():
        main(last % 2, 1 - last % 2, do_conv=False, do_stage=False)


@jax.jit
def pallas_standalone__window_attn_davit__vision_kernel(x, dw_pe, w_qkv, w_o):
    B, H, W, C = x.shape
    assert B == 1 and H % _WS == 0 and W % _WS == 0 and W + _WS + 1 <= 520 and C == 192
    nstrips = H // _WS
    WP = 512
    u32 = jnp.uint32
    xt = jnp.transpose(x, (0, 1, 3, 2)).reshape(H, C, W)
    dw = jnp.pad(dw_pe.reshape(9, C), ((0, 7), (0, 256 - C)))
    kern = functools.partial(_kernel, H=H, W=W, C=C, nstrips=nstrips)

    def strip(t):
        return jnp.minimum(t, nstrips - 1)

    out = pl.pallas_call(
        kern,
        grid=(nstrips + 2,),
        in_specs=[
            pl.BlockSpec((_WS, C, WP), lambda t: (strip(t), 0, 0)),
            pl.BlockSpec((1, C, WP), lambda t: (jnp.maximum(strip(t) * _WS - 1, 0), 0, 0)),
            pl.BlockSpec((1, C, WP), lambda t: (jnp.minimum(strip(t) * _WS + _WS, H - 1), 0, 0)),
            pl.BlockSpec((16, 256), lambda t: (0, 0)),
            pl.BlockSpec((C, 3 * C), lambda t: (0, 0)),
            pl.BlockSpec((C, C), lambda t: (0, 0)),
        ],
        out_specs=pl.BlockSpec((_WS, C, WP), lambda t: (jnp.maximum(t - 2, 0), 0, 0)),
        out_shape=jax.ShapeDtypeStruct((H, C, W), x.dtype),
        scratch_shapes=[
            pltpu.VMEM((9, C, 128), _F32),
            pltpu.VMEM((96, 256), u32),
            pltpu.VMEM((96, 256), u32),
            pltpu.VMEM((128, 256), u32),
            pltpu.VMEM((C // 2, 128), u32),
            pltpu.VMEM((C // 2, 128), u32),
            pltpu.VMEM((2, _WS + 2, C, WP), _F32),
            pltpu.VMEM((2, _WS, WP // 128, C, 128), _F32),
            pltpu.VMEM((2, 2, _WS, WP + 8, 128), _F32),
            pltpu.VMEM((2, 2, _WS, WP + 8, 128), _F32),
            pltpu.VMEM((_WS, WP + 8, 128), _F32),
            pltpu.VMEM((_WS, WP + 8, 128), _F32),
        ],
        compiler_params=pltpu.CompilerParams(
            dimension_semantics=("arbitrary",),
            vmem_limit_bytes=64 * 1024 * 1024,
        ),
    )(xt, xt, xt, dw, w_qkv, w_o)
    return jnp.transpose(out.reshape(1, H, C, W), (0, 1, 3, 2))
```

```python
import functools

import jax
import jax.numpy as jnp
import jax.experimental.pallas as pl
import jax.experimental.pallas.tpu as pltpu
import numpy as np

_WS = 7
_NH = 4
_NN = (((1,), (0,)), ((), ()))
_NT = (((1,), (1,)), ((), ()))
_F32 = jnp.float32
_BF16 = jnp.bfloat16
_NEG = -1e30
_GROUP = 2
_CH = 48
_CSPAN = 14
_NORM0, _NSPAN, _NLAG = 1, 26, 1
_ODIV = 7
_S0, _SSPAN = -1, 9
_ORDER = "ScVPnRos"


def _dot(a, b, dims):
    return jax.lax.dot_general(a, b, dims, preferred_element_type=_F32)


def _xpose(a):
    r, c = a.shape
    rp, cp = -(-r // 128) * 128, -(-c // 128) * 128
    if rp != r:
        a = jnp.concatenate([a, jnp.zeros((rp - r, c), a.dtype)], axis=0)
    if cp != c:
        a = jnp.concatenate([a, jnp.zeros((rp, cp - c), a.dtype)], axis=1)
    return a.T[:c, :r]


def _pk(a):
    return pltpu.bitcast(a.astype(_BF16), jnp.uint32)


def _upk(a):
    return pltpu.bitcast(a, _BF16)


def _kernel(x_ref, xu_ref, xd_ref, dw_ref, wqkv_ref, wo_ref, o_ref,
            wconv_s, lab_s, lba_s, rk_s, loe_s, loo_s,
            xs_s, x0_s, h_s, k_s, oe_s, oo_s, *, H, W, C, nstrips):
    t = pl.program_id(0)
    dh = C // _NH
    WP = 512
    nwin = W // _WS
    npair = (nwin + 1) // 2
    CH = _CH
    nunit = _WS * (C // CH)

    @pl.when(t == 0)
    def _prep():
        def padk(a):
            return jnp.concatenate([a, jnp.zeros((a.shape[0], 256 - C), _F32)], axis=1)
        wT = _xpose(wqkv_ref[...].astype(_F32))
        lab_s[...] = _pk(padk(jnp.concatenate(
            [wT[0:dh], wT[2 * dh:3 * dh], wT[2 * C:2 * C + 2 * dh]], axis=0)))
        lba_s[...] = _pk(padk(jnp.concatenate(
            [wT[dh:2 * dh], wT[3 * dh:4 * dh], wT[2 * C + 2 * dh:3 * C]], axis=0)))
        z = jnp.zeros((128 - 2 * dh, C), _F32)
        kscale = float(dh) ** -0.5 * float(np.log2(np.e))
        k01 = jnp.concatenate([wT[C:C + 2 * dh] * kscale, z], axis=0)
        k23 = jnp.concatenate([wT[C + 2 * dh:2 * C] * kscale, z], axis=0)
        rk_s[...] = _pk(jnp.concatenate([padk(k01).T, padk(k23).T], axis=1))
        wo = wo_ref[...].astype(_F32)
        woe = jnp.concatenate([wo[0:dh], wo[2 * dh:3 * dh], z], axis=0)
        woo = jnp.concatenate([wo[dh:2 * dh], wo[3 * dh:4 * dh], z], axis=0)
        loe_s[...] = _pk(_xpose(woe))
        loo_s[...] = _pk(_xpose(woo))
        dwT = _xpose(dw_ref[...].astype(_F32))
        for k in range(9):
            wk = jnp.broadcast_to(dwT[0:C, k:k + 1], (C, 128))
            wconv_s[k] = wk + 1.0 if k == 4 else wk
        h_s[:, :, :, pl.ds(WP, 8), :] = jnp.zeros((2, 2, _WS, 8, 128), _F32)
        k_s[:, :, :, pl.ds(WP, 8), :] = jnp.zeros((2, 2, _WS, 8, 128), _F32)

    def main(bufB, bufA, do_att=True, do_conv=True, do_stage=True):
        lane = jax.lax.broadcasted_iota(jnp.int32, (1, 128), 1)
        last_ok = lane < (W - (WP - 128))

        def stage_row(dst, ref, ok, src=0):
            v = ref[src].astype(_F32)
            okl = last_ok if ok is None else jnp.logical_and(last_ok, ok)
            lo = v[:, :WP - 128] if ok is None else jnp.where(ok, v[:, :WP - 128], 0.0)
            xs_s[bufB, dst, :, :WP - 128] = lo
            xs_s[bufB, dst, :, WP - 128:] = jnp.where(okl, v[:, WP - 128:], 0.0)

        def conv_unit(u):
            r = u // (C // CH)
            c0 = (u - r * (C // CH)) * CH
            y = [None, None, None]
            for a in range(3):
                xv = xs_s[bufA, r + a, c0:c0 + CH, :]
                for b in range(3):
                    w = wconv_s[3 * a + b, c0:c0 + CH, :]
                    term = xv * jnp.concatenate([w] * (WP // 128), axis=1)
                    y[b] = term if y[b] is None else y[b] + term
            x0 = y[1] + (pltpu.roll(y[0], 1, 1) + pltpu.roll(y[2], WP - 1, 1))
            for j in range(WP // 128):
                x0_s[bufA, r, j, c0:c0 + CH, :] = x0[:, 128 * j:128 * (j + 1)]

        def norm_unit(r, j):
            x0 = x0_s[bufA, r, j]
            mean = jnp.sum(x0, axis=0, keepdims=True) * (1.0 / C)
            ex2 = jnp.sum(x0 * x0, axis=0, keepdims=True) * (1.0 / C)
            rstd = jax.lax.rsqrt(jnp.maximum(ex2 - mean * mean, 0.0) + 1e-5)
            hn = (x0 - mean) * rstd
            hb = jnp.concatenate([hn, jnp.zeros((256 - C, 128), _F32)], axis=0).astype(_BF16).T
            hf = hb.astype(_F32)
            h_s[bufA, 0, r, 128 * j:128 * (j + 1), :] = hf[:, 0:128]
            h_s[bufA, 1, r, 128 * j:128 * (j + 1), :] = hf[:, 128:256]
            kk = _dot(hb, _upk(rk_s[...]), _NN)
            k_s[bufA, 0, r, 128 * j:128 * (j + 1), :] = kk[:, 0:128]
            k_s[bufA, 1, r, 128 * j:128 * (j + 1), :] = kk[:, 128:256]

        def out_unit(r, j):
            sl = slice(128 * j, 128 * (j + 1))
            oe = oe_s[r, sl, :].astype(_BF16)
            oo = oo_s[r, sl, :].astype(_BF16)
            for m in range(2):
                a0, b0 = 48 * m, 96 * m
                y = (_dot(_upk(loe_s[a0:a0 + 48, :]), oe, _NT) + _dot(_upk(loo_s[a0:a0 + 48, :]), oo, _NT))
                o_ref[r, b0:b0 + 96, sl] = (x0_s[bufB, r, j, b0:b0 + 96, :] + y).astype(o_ref.dtype)

        left = lane < 64
        qv, pr = {}, {}

        def selL(a):
            return jnp.where(left, a, 0.0)

        def selR(a):
            return jnp.where(left, 0.0, a)

        key_ok = (jax.lax.broadcasted_iota(jnp.int32, (56, 128), 0) % 8) < _WS
        z8 = jnp.zeros((8, 256), _F32)
        z32 = jnp.zeros((32, 128), _F32)
        z8l = jnp.zeros((8, 128), _F32)

        def softmax_t(s):
            s = jnp.where(key_ok, s, _NEG)
            m = jnp.max(s, axis=0, keepdims=True)
            p = jnp.exp2(s - m)
            l = jnp.sum(p, axis=0, keepdims=True)
            r0 = pl.reciprocal(l, approx=True)
            r1 = r0 * (2.0 - l * r0)
            return p, r1 * (2.0 - l * r1)

        def gather(ref, t0):
            return [jnp.concatenate([ref[bufB, k, r, pl.ds(t0, 8), :] for r in range(_WS)], axis=0)
                    for k in range(2)]

        def proj(p, slot):
            ta_ = p * (2 * _WS)
            hA = jnp.concatenate(gather(h_s, ta_), axis=1)
            hB = jnp.concatenate(gather(h_s, ta_ + _WS), axis=1)
            hAB = jnp.concatenate([hA, z8, hB, z8], axis=0).astype(_BF16)
            hBA = jnp.concatenate([hB, z8, hA, z8], axis=0).astype(_BF16)
            r1 = _dot(_upk(lab_s[...]), hAB, _NT)
            r2 = _dot(_upk(lba_s[...]), hBA, _NT)
            qs = []
            for t2 in range(2):
                e = r1[dh * t2:dh * (t2 + 1)]
                o = r2[dh * t2:dh * (t2 + 1)]
                qs.append(jnp.concatenate([selL(e), selR(o)], axis=0).astype(_BF16))
                qs.append(jnp.concatenate([selR(e), selL(o)], axis=0).astype(_BF16))
            vs = [a[k * dh:(k + 1) * dh].astype(_BF16) for a in (r1, r2) for k in (2, 3)]
            qv[p] = (qs, vs)

        def scores(p, slot):
            ta_ = p * (2 * _WS)
            kA = gather(k_s, ta_)
            kB = gather(k_s, ta_ + _WS)
            out = []
            for t2 in range(2):
                sA = _dot(kA[t2][:, 0:96], qv[p][0][2 * t2], _NN)
                sB = _dot(kB[t2][:, 0:96], qv[p][0][2 * t2 + 1], _NN)
                out.append((sA, sB))
            return out

        def probs(ss, slot):
            out = []
            for t2 in range(2):
                pA, rA = softmax_t(ss[t2][0])
                pB, rB = softmax_t(ss[t2][1])
                pe, po = [selL(pA), z8l, selR(pB), z8l], [selR(pA), z8l, selL(pB), z8l]
                if t2 == 1:
                    pe, po = pe[2:] + pe[:2], po[2:] + po[:2]
                out.append((jnp.concatenate(pe, axis=0).astype(_BF16),
                            jnp.concatenate(po, axis=0).astype(_BF16),
                            jnp.where(left, rA, rB), jnp.where(left, rB, rA)))
            pr[slot] = out

        def pv(p, slot):
            ta_ = p * (2 * _WS)
            tb_ = ta_ + _WS
            oe, oo = [], []
            for t2 in range(2):
                pe, po, re_, ro_ = pr[p][t2]
                oe.append(_dot(qv[p][1][2 * t2], pe, _NN) * re_)
                oo.append(_dot(qv[p][1][2 * t2 + 1], po, _NN) * ro_)
            oeT = jnp.concatenate(oe + [z32], axis=0).astype(_BF16).T.astype(_F32)
            ooT = jnp.concatenate(oo + [z32], axis=0).astype(_BF16).T.astype(_F32)
            for r in range(_WS):
                oe_s[r, pl.ds(ta_, 8), :] = oeT[8 * r:8 * r + 8]
                oo_s[r, pl.ds(ta_, 8), :] = ooT[64 + 8 * r:64 + 8 * r + 8]
            for r in range(_WS):
                oe_s[r, pl.ds(tb_, 8), :] = oeT[64 + 8 * r:64 + 8 * r + 8]
                oo_s[r, pl.ds(tb_, 8), :] = ooT[8 * r:8 * r + 8]

        G = _GROUP
        ngrp = -(-npair // G)
        ntile = WP // 128

        def members(g):
            return [(p, p) for p in range(g * G, min((g + 1) * G, npair))]

        side = {(k, g): [] for k in "cnos" for g in range(-1, ngrp)}
        conv_at = [-1 + (u * _CSPAN) // nunit for u in range(nunit)]
        conv_done = conv_at[-1] if do_conv else -2
        for u in range(nunit if do_conv else 0):
            side["c", conv_at[u]].append(functools.partial(conv_unit, u))
        nnorm = _WS * ntile
        for n in range(nnorm if do_conv else 0):
            r = n // ntile
            ready = conv_at[(C // CH) * (r + 1) - 1]
            g = max(ready + _NLAG, _NORM0 + (n * _NSPAN) // nnorm)
            side["n", min(g, ngrp - 1)].append(functools.partial(norm_unit, r, n % ntile))
        for j in range(ntile if do_att else 0):
            ready = min((128 * (j + 1) - 1) // (2 * _WS), npair - 1) // G
            nxt = min((128 * (j + 2) - 1) // (2 * _WS), npair - 1) // G if j + 1 < ntile else ready
            for r in range(_WS):
                g = ready + 1 + (r * (nxt - ready)) // _ODIV
                if g <= ngrp - 1:
                    side["o", g].append(functools.partial(out_unit, r, j))
        stages = [functools.partial(stage_row, 0, xu_ref, t > 0),
                  functools.partial(stage_row, _WS + 1, xd_ref, t < nstrips - 1)]
        stages += [functools.partial(stage_row, r + 1, x_ref, None, r) for r in range(_WS)]
        for n, fn in enumerate(stages if do_stage else []):
            g = _S0 + (n * _SSPAN) // len(stages)
            g = g if do_att else -1
            side["s", min(g, ngrp - 1)].append(fn)

        def step(g):
            ss = []
            sc = members(g + 1) if do_att and g + 1 < ngrp else []
            for c in _ORDER:
                if c == "S":
                    ss = [scores(p, sl) for p, sl in sc]
                elif c == "V" and do_att and g >= 0:
                    for p, sl in members(g):
                        pv(p, sl)
                elif c == "P" and do_att and g + 2 < ngrp:
                    for p, sl in members(g + 2):
                        proj(p, sl)
                elif c == "R":
                    for s_, (p, sl) in zip(ss, sc):
                        probs(s_, sl)
                elif c in "cnos":
                    for fn in side[c, g]:
                        fn()

        if do_att:
            for p, sl in members(0):
                proj(p, sl)
        for g in range(-1, ngrp):
            step(g)
        if do_att:
            for r in range(_WS):
                out_unit(r, ntile - 1)

    last = nstrips + 1
    parity = jax.lax.rem(t, 2)
    steady = jnp.logical_and(t >= 2, t < last)

    @pl.when(t == 0)
    def _first():
        main(0, 1, do_att=False, do_conv=False)

    @pl.when(t == 1)
    def _second():
        main(1, 0, do_att=False)

    @pl.when(jnp.logical_and(steady, parity == 0))
    def _even():
        main(0, 1)

    @pl.when(jnp.logical_and(steady, parity == 1))
    def _odd():
        main(1, 0)

    @pl.when(t == last)
    def _last():
        main(last % 2, 1 - last % 2, do_conv=False, do_stage=False)


@jax.jit
def pallas_standalone__window_attn_davit__vision_kernel(x, dw_pe, w_qkv, w_o):
    B, H, W, C = x.shape
    assert B == 1 and H % _WS == 0 and W % _WS == 0 and W + _WS + 1 <= 520 and C == 192
    nstrips = H // _WS
    WP = 512
    u32 = jnp.uint32
    xt = jnp.transpose(x, (0, 1, 3, 2)).reshape(H, C, W)
    dw = jnp.pad(dw_pe.reshape(9, C), ((0, 7), (0, 256 - C)))
    kern = functools.partial(_kernel, H=H, W=W, C=C, nstrips=nstrips)

    def strip(t):
        return jnp.minimum(t, nstrips - 1)

    out = pl.pallas_call(
        kern,
        grid=(nstrips + 2,),
        in_specs=[
            pl.BlockSpec((_WS, C, WP), lambda t: (strip(t), 0, 0)),
            pl.BlockSpec((1, C, WP), lambda t: (jnp.maximum(strip(t) * _WS - 1, 0), 0, 0)),
            pl.BlockSpec((1, C, WP), lambda t: (jnp.minimum(strip(t) * _WS + _WS, H - 1), 0, 0)),
            pl.BlockSpec((16, 256), lambda t: (0, 0)),
            pl.BlockSpec((C, 3 * C), lambda t: (0, 0)),
            pl.BlockSpec((C, C), lambda t: (0, 0)),
        ],
        out_specs=pl.BlockSpec((_WS, C, WP), lambda t: (jnp.maximum(t - 2, 0), 0, 0)),
        out_shape=jax.ShapeDtypeStruct((H, C, W), x.dtype),
        scratch_shapes=[
            pltpu.VMEM((9, C, 128), _F32),
            pltpu.VMEM((96, 256), u32),
            pltpu.VMEM((96, 256), u32),
            pltpu.VMEM((128, 256), u32),
            pltpu.VMEM((C // 2, 128), u32),
            pltpu.VMEM((C // 2, 128), u32),
            pltpu.VMEM((2, _WS + 2, C, WP), _F32),
            pltpu.VMEM((2, _WS, WP // 128, C, 128), _F32),
            pltpu.VMEM((2, 2, _WS, WP + 8, 128), _F32),
            pltpu.VMEM((2, 2, _WS, WP + 8, 128), _F32),
            pltpu.VMEM((_WS, WP + 8, 128), _F32),
            pltpu.VMEM((_WS, WP + 8, 128), _F32),
        ],
        compiler_params=pltpu.CompilerParams(
            dimension_semantics=("arbitrary",),
            vmem_limit_bytes=64 * 1024 * 1024,
        ),
    )(xt, xt, xt, dw, w_qkv, w_o)
    return jnp.transpose(out.reshape(1, H, C, W), (0, 1, 3, 2))
```
